```python
import jax
import jax.numpy as jnp

def _softmax(x, axis=-1):
    return jax.nn.softmax(x, axis=axis)

def _gelu(x):
    return jax.nn.gelu(x, approximate=True)

def _silu(x):
    return jax.nn.silu(x)

def _sigmoid(x):
    return jax.nn.sigmoid(x)

def _layernorm(x, axis=-1, eps=1e-05):
    m = jnp.mean(x, axis=axis, keepdims=True)
    v = jnp.var(x, axis=axis, keepdims=True)
    return (x - m) / jnp.sqrt(v + eps)

def _scatter_add(tgt, idx, src, axis=0):
    return tgt.at[idx].add(src)

def _segment_sum(src, seg, n):
    return jax.ops.segment_sum(src, seg, n)

class _Rng:

    def __init__(self, key):
        self._k = key

    def _next(self):
        self._k, sub = jax.random.split(self._k)
        return sub

    def normal(self, shape):
        return jax.random.normal(self._next(), shape, dtype=jnp.bfloat16)

    def randint(self, lo, hi, shape):
        return jax.random.randint(self._next(), shape, lo, hi, dtype=jnp.int32)

    def uniform(self, shape, lo=0.0, hi=1.0):
        return jax.random.uniform(self._next(), shape, jnp.bfloat16, lo, hi)

    def permutation(self, n):
        return jax.random.permutation(self._next(), n)
kernel_name = 'recurrent_scan__ssm_conv_h3__mixer_gmlp__prompt'

def setup_inputs():
    _rng = _Rng(jax.random.key(int.from_bytes(__import__("os").urandom(4), "little")))
    _w = lambda a: (lambda t: t.astype(jnp.bfloat16) if jnp.issubdtype(t.dtype, jnp.floating) else t)(jnp.asarray(a))

    def _A_setup():
        B, S, D = (1, 2048, 640)
        ks = 4
        return {'q': _w((lambda *s: _rng.normal(s) * 0.05)(B, S, D)), 'k': _w((lambda *s: _rng.normal(s) * 0.05)(B, S, D)), 'v': _w((lambda *s: _rng.normal(s) * 0.05)(B, S, D)), 'shift_k': _w((lambda *s: _rng.normal(s) * 0.05)(D, ks) * 0.5), 'ssm_k': _w((lambda *s: _rng.normal(s) * 0.05)(D, S) * (1.0 / S ** 0.5)), 'ssm_D': _w((lambda *s: _rng.normal(s) * 0.05)(D))}
    _A_in = _A_setup()

    def _B_setup():
        B, S, D, F = (1, 2048, 640, 1536)
        Fh = F // 2
        return {'x': _w((lambda *s: _rng.normal(s) * 0.05)(B, S, D)), 'w_in': _w((lambda *s: _rng.normal(s) * 0.05)(D, 2 * Fh)), 'w_sp': _w(0.01 * (lambda *s: _rng.normal(s) * 0.05)(S, S)), 'b_sp': _w(1.0 + 0.01 * (lambda *s: _rng.normal(s) * 0.05)(S)), 'w_out': _w((lambda *s: _rng.normal(s) * 0.05)(Fh, D))}
    _B_in = _B_setup()
    return {'A_q': _A_in['q'], 'A_k': _A_in['k'], 'A_v': _A_in['v'], 'A_shift_k': _A_in['shift_k'], 'A_ssm_k': _A_in['ssm_k'], 'A_ssm_D': _A_in['ssm_D'], 'B_x': _B_in['x'], 'B_w_in': _B_in['w_in'], 'B_w_sp': _B_in['w_sp'], 'B_b_sp': _B_in['b_sp'], 'B_w_out': _B_in['w_out']}

def reference(A_q, A_k, A_v, A_shift_k, A_ssm_k, A_ssm_D, B_x, B_w_in, B_w_sp, B_b_sp, B_w_out):

    def _A_ref(q, k, v, shift_k, ssm_k, ssm_D):
        B, S, D = q.shape
        ks = shift_k.shape[-1]
        k_pad = jnp.pad(k, ((0, 0), (ks - 1, 0), (0, 0)))
        k_shift = jnp.zeros_like(k)
        for t in range(ks):
            k_shift = k_shift + k_pad[:, t:t + S, :] * shift_k[:, ks - 1 - t][None, None, :]
        kv = k_shift * v
        L = 2 * S
        kv_pad = jnp.pad(kv, ((0, 0), (0, S), (0, 0)))
        kf_pad = jnp.pad(ssm_k, ((0, 0), (0, S)))
        kv_f = (lambda x, axes=(-2, -1): jnp.fft.rfft2(x.astype(jnp.float32), axes=axes))(kv_pad[:, None, :, :], axes=(1, 2))
        kf_f = (lambda x, axes=(-2, -1): jnp.fft.rfft2(x.astype(jnp.float32), axes=axes))(kf_pad[:, None, :], axes=(1, 2))
        kf_f = (lambda x, *d: x.transpose(*d))(kf_f, 1, 2, 0)
        y_f = kv_f * kf_f[None, :, :, :]
        y = (lambda x, s, axes=(-2, -1): jnp.fft.irfft2(x, s=s, axes=axes).astype(jnp.bfloat16))(y_f, (1, L), axes=(1, 2))[:, 0, :S, :]
        y = y + kv * ssm_D[None, None, :]
        return q * y

    def _B_ref(x, w_in, w_sp, b_sp, w_out):
        B, S, D = x.shape
        F = w_in.shape[-1]
        Fh = F // 2
        z = _gelu(jnp.einsum('bsd,df->bsf', x, w_in))
        z1 = z[..., :Fh].copy()
        z2 = _layernorm(z[..., Fh:], axis=-1)
        g = jnp.einsum('ts,bsf->btf', w_sp, z2) + b_sp[None, :, None]
        return jnp.einsum('bsf,fd->bsd', z1 * g, w_out)
    x = A_q
    xn = _layernorm(x, axis=-1)
    s = _A_ref(xn, A_k, A_v, A_shift_k, A_ssm_k, A_ssm_D)
    g = _silu(_B_ref(xn, B_w_in, B_w_sp, B_b_sp, B_w_out))
    return x + s * g
```

```python
import functools
import os

import jax
import jax.numpy as jnp
import numpy as np
import jax.experimental.pallas as pl
import jax.experimental.pallas.tpu as pltpu

_C = 128
_TM1 = int(os.environ.get('TM1', 256))
_TM2 = int(os.environ.get('TM2', 128))
_TM3 = int(os.environ.get('TM3', 256))
_KC = int(os.environ.get('KC', 512))


def _dft_matrix():
    c = _C
    f = np.concatenate([np.arange(0, c, 2), np.arange(1, c, 2)])
    t = np.arange(c)
    m = ((2 * f[:, None] + 1) * t[None, :]) % (4 * c)
    th = np.pi * m.astype(np.float64) / (2 * c)
    return np.concatenate([np.cos(th), -np.sin(th)], axis=0)


_F_NP = _dft_matrix()


def _ln(x):
    m = jnp.mean(x, axis=-1, keepdims=True)
    xc = x - m
    v = jnp.mean(xc * xc, axis=-1, keepdims=True)
    return xc * jax.lax.rsqrt(v + 1e-5)


def _gelu(x):
    c0 = 0.7978845608028654
    return 0.5 * x * (1.0 + jnp.tanh(c0 * (x + 0.044715 * x * x * x)))


def _silu(x):
    return 0.5 * x * (1.0 + jnp.tanh(0.5 * x))


def _pack(x):
    return pltpu.bitcast(x, jnp.uint32)


def _unpack(x):
    return pltpu.bitcast(x, jnp.bfloat16)


def _kernel(x_hbm, k_hbm, v_hbm, shk_hbm, h_hbm, d_hbm, win_hbm, wsp_hbm, b_hbm, wout_hbm, f_hbm, g_hbm,
            o_hbm,
            x_v, k_v, v_v, shk_v, h_v, d_v, win_v, wsp_v, b_v, wout_v, f_v, g_v,
            xn_s, kv_s, z1_s, z2_s, gate_s, u_s, hh_s, y_s, o_s, p_s,
            sem_t, sem_m, sem_o,
            *, S, D, FH):
    C, TM1, TM2, TM3, KC = _C, _TM1, _TM2, _TM3, _KC
    NT1, NT2, NT3 = S // TM1, S // TM2, S // TM3
    NB = S // C
    f32, bf16 = jnp.float32, jnp.bfloat16

    def rows(i, n):
        return pl.ds(pl.multiple_of(i * n, n), n)

    def tile_copies(i):
        r = rows(i, TM1)
        return [
            pltpu.make_async_copy(x_hbm.at[r], x_v.at[r], sem_t.at[0, i]),
            pltpu.make_async_copy(k_hbm.at[r], k_v.at[pl.ds(pl.multiple_of(i * TM1 + 16, 16), TM1)], sem_t.at[1, i]),
            pltpu.make_async_copy(v_hbm.at[r], v_v.at[r], sem_t.at[2, i]),
            pltpu.make_async_copy(h_hbm.at[:, r], h_v.at[:, r], sem_t.at[3, i]),
        ]

    def wsp_copy(i):
        r = rows(i, TM1)
        return pltpu.make_async_copy(wsp_hbm.at[r], wsp_v.at[r], sem_t.at[4, i])

    misc = [
        pltpu.make_async_copy(win_hbm, win_v, sem_m.at[0]),
        pltpu.make_async_copy(shk_hbm, shk_v, sem_m.at[1]),
        pltpu.make_async_copy(f_hbm, f_v, sem_m.at[2]),
        pltpu.make_async_copy(d_hbm, d_v, sem_m.at[3]),
        pltpu.make_async_copy(b_hbm, b_v, sem_m.at[4]),
        pltpu.make_async_copy(wout_hbm, wout_v, sem_m.at[5]),
        pltpu.make_async_copy(g_hbm, g_v, sem_m.at[6]),
    ]

    t0 = tile_copies(0)
    t0[0].start()
    misc[0].start()
    misc[1].start()
    misc[2].start()
    for c in t0[1:]:
        c.start()
    k_v[pl.ds(0, 16), :] = jnp.zeros((16, D), bf16)
    misc[0].wait()
    misc[1].wait()
    misc[2].wait()

    def p1(i, carry):
        @pl.when(i + 1 < NT1)
        def _():
            for c in tile_copies(i + 1):
                c.start()

        @pl.when(i == 1)
        def _():
            for c in misc[3:]:
                c.start()

        @pl.when(i >= 1)
        def _():
            wsp_copy(i - 1).start()

        for c in tile_copies(i):
            c.wait()
        r = rows(i, TM1)
        rh = rows(i, TM1 // 2)
        r0 = pl.multiple_of(i * TM1, TM1)
        xn = _ln(x_v[r, :].astype(f32)).astype(bf16)
        xn_s[rh, :] = _pack(xn)
        z = _gelu(jnp.dot(xn, win_v[...], preferred_element_type=f32))
        z1_s[rh, :] = _pack(z[:, :FH].astype(bf16))
        z2_s[rh, :] = _pack(_ln(z[:, FH:]).astype(bf16))
        kk = k_v[pl.ds(r0, TM1 + 16), :].astype(f32)
        shk = shk_v[...].astype(f32)
        ks = kk[16:16 + TM1] * shk[0:1, :]
        for j in range(1, 4):
            ks = ks + kk[16 - j:16 - j + TM1] * shk[j:j + 1, :]
        kv = (ks * v_v[r, :].astype(f32)).astype(bf16)
        kv_s[rh, :] = _pack(kv)
        fm = f_v[...]
        for bb in range(TM1 // C):
            b = i * (TM1 // C) + bb
            u_s[b] = jnp.dot(fm, kv[bb * C:(bb + 1) * C, :], preferred_element_type=f32)
            hb = h_v[:, pl.ds(pl.multiple_of(r0 + bb * C, C), C)]
            hh_s[b] = jax.lax.dot_general(fm, hb, (((1,), (1,)), ((), ())), preferred_element_type=f32)
        return carry

    jax.lax.fori_loop(0, NT1, p1, 0)
    wsp_copy(NT1 - 1).start()
    for c in misc[3:]:
        c.wait()
    for i in range(NT1):
        wsp_copy(i).wait()

    NLT = D // 128
    FPS = C // NT2
    dep = []

    def conv_gen(fr0, never):
        sgn = jnp.where(fr0 < C // 2, 1.0, -1.0).astype(f32)
        for c in range(NLT):
            ls = slice(c * 128, (c + 1) * 128)
            for half in range(FPS // 8):
                fre = pl.ds(pl.multiple_of(fr0 + half * 8, 8), 8)
                fim = pl.ds(pl.multiple_of(fr0 + half * 8 + C, 8), 8)
                prev = None
                for b in range(NB):
                    ar = ai = None
                    for m in range(b + 1):
                        hr = hh_s[m, fre, ls]
                        if dep:
                            hr = jnp.where(never, dep.pop(), hr)
                        hi = hh_s[m, fim, ls]
                        ur = u_s[b - m, fre, ls]
                        ui = u_s[b - m, fim, ls]
                        pr = hr * ur - hi * ui
                        pi = hr * ui + hi * ur
                        ar = pr if ar is None else ar + pr
                        ai = pi if ai is None else ai + pi
                        yield
                    if prev is None:
                        yr, yi = ar, ai
                    else:
                        yr = ar - sgn * prev[1]
                        yi = ai + sgn * prev[0]
                    prev = (ar, ai)
                    y_s[b, fre, ls] = yr
                    y_s[b, fim, ls] = yi

    NPAIR = NLT * (FPS // 8) * (NB * (NB + 1) // 2)

    def p2(i, carry):
        r = rows(i, TM2)
        rh = rows(i, TM2 // 2)
        never = jax.lax.broadcasted_iota(jnp.int32, (8, 128), 0) > (i + 8)
        gen = conv_gen(i * FPS, never)
        npieces = (FH // 128) * (S // KC) + D // 128
        per = -(-NPAIR // npieces)

        def pump(d):
            dep.append(d[0:8, 0:128])
            for _ in range(per):
                next(gen, None)

        bias = b_v[r, :].astype(f32)
        for n in range(FH // 128):
            ns = slice(n * 128, (n + 1) * 128)
            acc = None
            for kc in range(S // KC):
                d = jnp.dot(wsp_v[r, kc * KC:(kc + 1) * KC], _unpack(z2_s[kc * KC // 2:(kc + 1) * KC // 2, ns]),
                            preferred_element_type=f32)
                acc = d if acc is None else acc + d
                pump(d)
            p_s[:, ns] = _pack((_unpack(z1_s[rh, ns]).astype(f32) * (acc + bias)).astype(bf16))
        p = _unpack(p_s[...])
        for n in range(D // 128):
            ns = slice(n * 128, (n + 1) * 128)
            o = jnp.dot(p, wout_v[:, ns], preferred_element_type=f32)
            gate_s[r, ns] = _silu(o)
            pump(o)
        for _ in gen:
            pass
        return carry

    jax.lax.fori_loop(0, NT2, p2, 0)

    def out_copy(i):
        r = rows(i, TM3)
        return pltpu.make_async_copy(o_s.at[r], o_hbm.at[r], sem_o.at[i])

    def p3(i, carry):
        gm = g_v[...]
        dd = d_v[...].astype(f32)
        for bb in range(TM3 // C):
            b = i * (TM3 // C) + bb
            rr = rows(b, C)
            rrh = rows(b, C // 2)
            y = jnp.dot(gm, y_s[b].astype(bf16), preferred_element_type=f32)
            y = y + _unpack(kv_s[rrh, :]).astype(f32) * dd
            s = _unpack(xn_s[rrh, :]).astype(f32) * y
            o_s[rr, :] = (x_v[rr, :].astype(f32) + s * gate_s[rr, :]).astype(bf16)
        out_copy(i).start()
        return carry

    jax.lax.fori_loop(0, NT3, p3, 0)
    for i in range(NT3):
        out_copy(i).wait()


@jax.jit
def pallas_recurrent_scan__ssm_conv_h3__mixer_gmlp__prompt_kernel(
    A_q: jax.Array,
    A_k: jax.Array,
    A_v: jax.Array,
    A_shift_k: jax.Array,
    A_ssm_k: jax.Array,
    A_ssm_D: jax.Array,
    B_x: jax.Array,
    B_w_in: jax.Array,
    B_w_sp: jax.Array,
    B_b_sp: jax.Array,
    B_w_out: jax.Array,
):
    del B_x
    _, S, D = A_q.shape
    F = B_w_in.shape[-1]
    FH = F // 2
    C = _C
    NB = S // C
    bf16, f32, u32 = jnp.bfloat16, jnp.float32, jnp.uint32

    x = A_q.reshape(S, D)
    k = A_k.reshape(S, D)
    v = A_v.reshape(S, D)
    shk = A_shift_k.T
    dvec = A_ssm_D.reshape(1, D)
    bvec = B_b_sp.reshape(S, 1)
    fmat = np.asarray(_F_NP, dtype=np.float32).astype(bf16)
    gmat = np.asarray(_F_NP.T / C, dtype=np.float32).astype(bf16)

    kern = functools.partial(_kernel, S=S, D=D, FH=FH)
    any_spec = pl.BlockSpec(memory_space=pl.ANY)
    out = pl.pallas_call(
        kern,
        out_shape=jax.ShapeDtypeStruct((S, D), bf16),
        in_specs=[any_spec] * 12,
        out_specs=any_spec,
        scratch_shapes=[
            pltpu.VMEM((S, D), bf16),
            pltpu.VMEM((S + 16, D), bf16),
            pltpu.VMEM((S, D), bf16),
            pltpu.VMEM(shk.shape, bf16),
            pltpu.VMEM((D, S), bf16),
            pltpu.VMEM((1, D), bf16),
            pltpu.VMEM((D, F), bf16),
            pltpu.VMEM((S, S), bf16),
            pltpu.VMEM((S, 1), bf16),
            pltpu.VMEM((FH, D), bf16),
            pltpu.VMEM((2 * C, C), bf16),
            pltpu.VMEM((C, 2 * C), bf16),
            pltpu.VMEM((S // 2, D), u32),
            pltpu.VMEM((S // 2, D), u32),
            pltpu.VMEM((S // 2, FH), u32),
            pltpu.VMEM((S // 2, FH), u32),
            pltpu.VMEM((S, D), f32),
            pltpu.VMEM((NB, 2 * C, D), f32),
            pltpu.VMEM((NB, 2 * C, D), f32),
            pltpu.VMEM((NB, 2 * C, D), f32),
            pltpu.VMEM((S, D), bf16),
            pltpu.VMEM((_TM2 // 2, FH), u32),
            pltpu.SemaphoreType.DMA((5, S // _TM1)),
            pltpu.SemaphoreType.DMA((7,)),
            pltpu.SemaphoreType.DMA((S // _TM3,)),
        ],
        compiler_params=pltpu.CompilerParams(vmem_limit_bytes=120 * 1024 * 1024),
    )(x, k, v, shk, A_ssm_k, dvec, B_w_in, B_w_sp, bvec, B_w_out, fmat, gmat)
    return out.reshape(1, S, D)
```

```python
import functools
import os

import jax
import jax.numpy as jnp
import numpy as np
import jax.experimental.pallas as pl
import jax.experimental.pallas.tpu as pltpu

_C = 128
_TM1 = int(os.environ.get('TM1', 256))
_TM2 = int(os.environ.get('TM2', 128))
_TM3 = int(os.environ.get('TM3', 512))
_KC = int(os.environ.get('KC', 256))


def _dft_matrix():
    c = _C
    f = np.concatenate([np.arange(0, c, 2), np.arange(1, c, 2)])
    t = np.arange(c)
    m = ((2 * f[:, None] + 1) * t[None, :]) % (4 * c)
    th = np.pi * m.astype(np.float64) / (2 * c)
    return np.concatenate([np.cos(th), -np.sin(th)], axis=0)


_F_NP = _dft_matrix()


def _ln(x):
    m = jnp.mean(x, axis=-1, keepdims=True)
    xc = x - m
    v = jnp.mean(xc * xc, axis=-1, keepdims=True)
    return xc * jax.lax.rsqrt(v + 1e-5)


def _gelu(x):
    c0 = 0.7978845608028654
    return 0.5 * x * (1.0 + jnp.tanh(c0 * (x + 0.044715 * x * x * x)))


def _silu(x):
    return 0.5 * x * (1.0 + jnp.tanh(0.5 * x))


def _pack(x):
    return pltpu.bitcast(x, jnp.uint32)


def _unpack(x):
    return pltpu.bitcast(x, jnp.bfloat16)


def _kernel(x_hbm, k_hbm, v_hbm, shk_hbm, h_hbm, d_hbm, win_hbm, wsp_hbm, b_hbm, wout_hbm, f_hbm, g_hbm,
            o_hbm,
            x_v, k_v, v_v, shk_v, h_v, d_v, win_v, wsp_v, b_v, wout_v, f_v, g_v,
            xn_s, kv_s, z1_s, z2_s, u_s, hh_s, y_s, o_s, p_s, bcol_s,
            sem_t, sem_m, sem_o,
            *, S, D, FH):
    C, TM1, TM2, TM3, KC = _C, _TM1, _TM2, _TM3, _KC
    NT1, NT2, NT3 = S // TM1, S // TM2, S // TM3
    NB = S // C
    f32, bf16 = jnp.float32, jnp.bfloat16

    def rows(i, n):
        return pl.ds(pl.multiple_of(i * n, n), n)

    def tile_copies(i):
        r = rows(i, TM1)
        return [
            None,
            pltpu.make_async_copy(k_hbm.at[r], k_v.at[pl.ds(pl.multiple_of(i * TM1 + 16, 16), TM1)], sem_t.at[1, i]),
            pltpu.make_async_copy(v_hbm.at[r], v_v.at[r], sem_t.at[2, i]),
            pltpu.make_async_copy(h_hbm.at[:, r], h_v.at[:, r], sem_t.at[3, i]),
        ]

    def wsp_copy(i):
        r = rows(i, TM1)
        return pltpu.make_async_copy(wsp_hbm.at[r], wsp_v.at[r], sem_t.at[4, i])

    misc = [
        pltpu.make_async_copy(win_hbm, win_v, sem_m.at[0]),
        pltpu.make_async_copy(shk_hbm, shk_v, sem_m.at[1]),
        pltpu.make_async_copy(f_hbm, f_v, sem_m.at[2]),
        pltpu.make_async_copy(d_hbm, d_v, sem_m.at[3]),
        pltpu.make_async_copy(b_hbm, b_v, sem_m.at[4]),
        pltpu.make_async_copy(wout_hbm, wout_v, sem_m.at[5]),
        pltpu.make_async_copy(g_hbm, g_v, sem_m.at[6]),
    ]

    x_copy = lambda i: pltpu.make_async_copy(x_hbm.at[rows(i, TM1)], x_v.at[rows(i, TM1)], sem_t.at[0, i])
    kvh_copies = lambda i: tile_copies(i)[1:]
    x_copy(0).start()
    misc[0].start()
    misc[1].start()
    misc[2].start()
    for c in kvh_copies(0):
        c.start()
    x_copy(1).start()
    k_v[pl.ds(0, 16), :] = jnp.zeros((16, D), bf16)
    with jax.named_scope("p0"):
        x_copy(0).wait()
    xn_s[rows(0, TM1 // 2), :] = _pack(_ln(x_v[rows(0, TM1), :].astype(f32)).astype(bf16))
    for c in misc[3:]:
        c.start()
    with jax.named_scope("p0b"):
        misc[0].wait()
        misc[1].wait()
        misc[2].wait()

    def p1(i, carry):
        @pl.when(i + 1 < NT1)
        def _():
            for c in kvh_copies(i + 1):
                c.start()
            x_copy(i + 1).wait()

        @pl.when(i + 2 < NT1)
        def _():
            x_copy(i + 2).start()

        wsp_copy(i).start()
        for c in kvh_copies(i):
            c.wait()
        r = rows(i, TM1)
        rh = rows(i, TM1 // 2)
        r0 = pl.multiple_of(i * TM1, TM1)
        never = jax.lax.broadcasted_iota(jnp.int32, (8, 128), 0) > (i + 8)

        def anchor(val, d):
            a0 = jnp.where(never, d[0:8, 0:128].astype(val.dtype), val[0:8, 0:128])
            top = jnp.concatenate([a0, val[8:, 0:128]], axis=0)
            return top if val.shape[1] == 128 else jnp.concatenate([top, val[:, 128:]], axis=1)

        never16 = jax.lax.broadcasted_iota(jnp.int32, (16, 128), 0) > (i + 16)
        pins = {}

        def pinned(lhs, j):
            if j not in pins:
                return lhs
            t = None
            for pv in pins[j]:
                for c0 in range(0, pv.shape[1], 128):
                    for rr0 in range(0, pv.shape[0], 8 * PST):
                        q = pv[rr0:rr0 + 8, c0:c0 + 128]
                        t = q if t is None else jnp.maximum(t, q)
            t = jnp.concatenate([t, t], axis=0).astype(bf16)
            cols = []
            for c0 in range(0, lhs.shape[1], 128):
                a0 = jnp.where(never16, t, lhs[0:16, c0:c0 + 128])
                cols.append(jnp.concatenate([a0, lhs[16:, c0:c0 + 128]], axis=0))
            return cols[0] if len(cols) == 1 else jnp.concatenate(cols, axis=1)

        PST = int(os.environ.get('PST', 1))
        PL = int(os.environ.get('PL', 4))
        NZ = FH // 128
        BPT = TM1 // C
        fm = f_v[...]
        xn = _unpack(xn_s[rh, :])
        shk = shk_v[...].astype(f32)
        j = 0
        z2 = []
        kvs = []
        KVP = eval(os.environ.get('KVP', '[3,3,5,12,13]'))

        def do_kv(n, anc):
            ls = slice(n * 128, (n + 1) * 128)
            kk = k_v[pl.ds(r0, TM1 + 16), ls].astype(f32)
            if anc is not None:
                kk = anchor(kk, anc)
            ks = kk[16:16 + TM1] * shk[0:1, ls]
            for t in range(1, 4):
                ks = ks + kk[16 - t:16 - t + TM1] * shk[t:t + 1, ls]
            kvn = ks * v_v[r, ls].astype(f32)
            pins.setdefault(KVP[n], []).append(kvn)
            kvn = kvn.astype(bf16)
            kv_s[rh, ls] = _pack(kvn)
            kvs.append(kvn)

        def do_h(bb):
            hb = h_v[:, pl.ds(pl.multiple_of(r0 + bb * C, C), C)]
            hh_s[i * BPT + bb] = jax.lax.dot_general(pinned(fm, j), hb, (((1,), (1,)), ((), ())),
                                                     preferred_element_type=f32)

        do_h(0)
        j += 1
        do_kv(0, None)
        do_kv(1, None)
        for n in range(NZ):
            d = jnp.dot(pinned(xn, j), win_v[:, FH + n * 128:FH + (n + 1) * 128], preferred_element_type=f32)
            gl = _gelu(d)
            z2.append(gl)
            pins.setdefault(j + PL, []).append(gl)
            if n == 1:
                do_kv(2, d)
            j += 1
        do_h(1)
        j += 1
        zl = _ln(jnp.concatenate(z2, axis=1))
        z2_s[rh, :] = _pack(zl.astype(bf16))
        pins.setdefault(j + 3, []).append(zl)
        for n in range(NZ):
            d = jnp.dot(pinned(xn, j), win_v[:, n * 128:(n + 1) * 128], preferred_element_type=f32)
            gl = _gelu(d)
            z1_s[rh, n * 128:(n + 1) * 128] = _pack(gl.astype(bf16))
            pins.setdefault(j + PL, []).append(gl)
            if n == 1:
                do_kv(3, d)
            if n == 2:
                do_kv(4, d)
            if n == 4:
                inx = jnp.minimum(i + 1, NT1 - 1)
                xx = _ln(anchor(x_v[rows(inx, TM1), :].astype(f32), d))
                xn_s[rows(inx, TM1 // 2), :] = _pack(xx.astype(bf16))
            j += 1
        kv = jnp.concatenate(kvs, axis=1)
        for bb in range(BPT):
            b = i * BPT + bb
            u_s[b] = jnp.dot(pinned(fm, j), kv[bb * C:(bb + 1) * C, :], preferred_element_type=f32)
            j += 1
        return carry

    with jax.named_scope('p1'):
        jax.lax.fori_loop(0, NT1, p1, 0)
    with jax.named_scope('p1b'):
        for c in misc[3:]:
            c.wait()
        for i in range(NT1):
            wsp_copy(i).wait()

    bcol_s[...] = jnp.broadcast_to(b_v[...].astype(f32).reshape(1, S), (128, S)).T

    NLT = D // 128
    FPS = C // NT2
    dep = []
    last = [None]
    PINW = int(os.environ.get('PINW', 128))
    LAG = int(os.environ.get('LAG', 3))

    def conv_gen(fr0, never):
        sgn = jnp.where(fr0 < C // 2, 1.0, -1.0).astype(f32)
        for c in range(NLT):
            ls = slice(c * 128, (c + 1) * 128)
            for half in range(FPS // 8):
                fre = pl.ds(pl.multiple_of(fr0 + half * 8, 8), 8)
                fim = pl.ds(pl.multiple_of(fr0 + half * 8 + C, 8), 8)
                prev = None
                for b in range(NB):
                    ar = ai = None
                    for m in range(b + 1):
                        hr = hh_s[m, fre, ls]
                        if dep:
                            hr = jnp.where(never, dep.pop(), hr)
                        hi = hh_s[m, fim, ls]
                        ur = u_s[b - m, fre, ls]
                        ui = u_s[b - m, fim, ls]
                        pr = hr * ur - hi * ui
                        pi = hr * ui + hi * ur
                        ar = pr if ar is None else ar + pr
                        ai = pi if ai is None else ai + pi
                        last[0] = ar
                        yield
                    if prev is None:
                        yr, yi = ar, ai
                    else:
                        yr = ar - sgn * prev[1]
                        yi = ai + sgn * prev[0]
                    prev = (ar, ai)
                    y_s[b, fre, ls] = yr
                    y_s[b, fim, ls] = yi
                    last[0] = yr

    NPAIR = NLT * (FPS // 8) * (NB * (NB + 1) // 2)

    def p2(i, carry):
        r = rows(i, TM2)
        rh = rows(i, TM2 // 2)
        never = jax.lax.broadcasted_iota(jnp.int32, (8, 128), 0) > (i + 8)
        gen = conv_gen(i * FPS, never)
        never16 = jax.lax.broadcasted_iota(jnp.int32, (16, 128), 0) > (i + 16)
        hist = []
        npieces = (FH // 128) * (S // KC)
        per = -(-NPAIR // npieces)

        def pump(d):
            dep.append(d[0:8, 0:128])
            for _ in range(per if not int(os.environ.get('NOCONV', 0)) else 1):
                next(gen, None)
            hist.append(last[0])

        bias = bcol_s[r, :]
        for n in range(FH // 128):
            ns = slice(n * 128, (n + 1) * 128)
            acc = None
            for kc in range(S // KC):
                lhs = wsp_v[r, kc * KC:(kc + 1) * KC]
                if LAG and len(hist) >= LAG:
                    t = jnp.concatenate([hist[-LAG]] * 2, axis=0).astype(bf16)
                    cols = []
                    for c0 in range(0, KC, 128):
                        if c0 < PINW:
                            a0 = jnp.where(never16, t, lhs[0:16, c0:c0 + 128])
                            cols.append(jnp.concatenate([a0, lhs[16:, c0:c0 + 128]], axis=0))
                        else:
                            cols.append(lhs[:, c0:c0 + 128])
                    lhs = cols[0] if len(cols) == 1 else jnp.concatenate(cols, axis=1)
                d = jnp.dot(lhs, _unpack(z2_s[kc * KC // 2:(kc + 1) * KC // 2, ns]),
                            preferred_element_type=f32)
                acc = d if acc is None else acc + d
                pump(d)
            p_s[rh, ns] = _pack((_unpack(z1_s[rh, ns]).astype(f32) * (acc + bias)).astype(bf16))
        if not int(os.environ.get('NOCONV', 0)):
            for _ in gen:
                pass
        return carry

    with jax.named_scope('p2'):
        jax.lax.fori_loop(0, NT2, p2, 0)

    def out_copy(i):
        r = rows(i, TM3)
        return pltpu.make_async_copy(o_s.at[r], o_hbm.at[r], sem_o.at[i])

    def p3(i, carry):
        gm = g_v[...]
        dd = d_v[...].astype(f32).reshape(1, D)
        gate = _silu(jnp.dot(_unpack(p_s[rows(i, TM3 // 2), :]), wout_v[...], preferred_element_type=f32))
        for bb in range(TM3 // C):
            b = i * (TM3 // C) + bb
            rr = rows(b, C)
            rrh = rows(b, C // 2)
            y = jnp.dot(gm, y_s[b].astype(bf16), preferred_element_type=f32)
            y = y + _unpack(kv_s[rrh, :]).astype(f32) * dd
            s = _unpack(xn_s[rrh, :]).astype(f32) * y
            o_s[rr, :] = (x_v[rr, :].astype(f32) + s * gate[bb * C:(bb + 1) * C]).astype(bf16)
        out_copy(i).start()
        return carry

    with jax.named_scope('p3'):
        jax.lax.fori_loop(0, NT3, p3, 0)
    with jax.named_scope('p4'):
        for i in range(NT3):
            out_copy(i).wait()


@jax.jit
def pallas_recurrent_scan__ssm_conv_h3__mixer_gmlp__prompt_kernel(
    A_q: jax.Array,
    A_k: jax.Array,
    A_v: jax.Array,
    A_shift_k: jax.Array,
    A_ssm_k: jax.Array,
    A_ssm_D: jax.Array,
    B_x: jax.Array,
    B_w_in: jax.Array,
    B_w_sp: jax.Array,
    B_b_sp: jax.Array,
    B_w_out: jax.Array,
):
    del B_x
    _, S, D = A_q.shape
    F = B_w_in.shape[-1]
    FH = F // 2
    C = _C
    NB = S // C
    bf16, f32, u32 = jnp.bfloat16, jnp.float32, jnp.uint32

    x = A_q.reshape(S, D)
    k = A_k.reshape(S, D)
    v = A_v.reshape(S, D)
    shk = A_shift_k.T
    dvec = A_ssm_D
    bvec = B_b_sp
    fmat = np.asarray(_F_NP, dtype=np.float32).astype(bf16)
    gmat = np.asarray(_F_NP.T / C, dtype=np.float32).astype(bf16)

    kern = functools.partial(_kernel, S=S, D=D, FH=FH)
    any_spec = pl.BlockSpec(memory_space=pl.ANY)
    out = pl.pallas_call(
        kern,
        out_shape=jax.ShapeDtypeStruct((S, D), bf16),
        in_specs=[any_spec] * 12,
        out_specs=any_spec,
        scratch_shapes=[
            pltpu.VMEM((S, D), bf16),
            pltpu.VMEM((S + 16, D), bf16),
            pltpu.VMEM((S, D), bf16),
            pltpu.VMEM(shk.shape, bf16),
            pltpu.VMEM((D, S), bf16),
            pltpu.VMEM((D,), bf16),
            pltpu.VMEM((D, F), bf16),
            pltpu.VMEM((S, S), bf16),
            pltpu.VMEM((S,), bf16),
            pltpu.VMEM((FH, D), bf16),
            pltpu.VMEM((2 * C, C), bf16),
            pltpu.VMEM((C, 2 * C), bf16),
            pltpu.VMEM((S // 2, D), u32),
            pltpu.VMEM((S // 2, D), u32),
            pltpu.VMEM((S // 2, FH), u32),
            pltpu.VMEM((S // 2, FH), u32),
            pltpu.VMEM((NB, 2 * C, D), f32),
            pltpu.VMEM((NB, 2 * C, D), f32),
            pltpu.VMEM((NB, 2 * C, D), f32),
            pltpu.VMEM((S, D), bf16),
            pltpu.VMEM((S // 2, FH), u32),
            pltpu.VMEM((S, 128), f32),
            pltpu.SemaphoreType.DMA((5, S // _TM1)),
            pltpu.SemaphoreType.DMA((7,)),
            pltpu.SemaphoreType.DMA((S // _TM3,)),
        ],
        compiler_params=pltpu.CompilerParams(vmem_limit_bytes=120 * 1024 * 1024),
    )(x, k, v, shk, A_ssm_k, dvec, B_w_in, B_w_sp, bvec, B_w_out, fmat, gmat)
    return out.reshape(1, S, D)
```

```python
import functools
import os

import jax
import jax.numpy as jnp
import numpy as np
import jax.experimental.pallas as pl
import jax.experimental.pallas.tpu as pltpu

_C = 128
_TM1 = int(os.environ.get('TM1', 256))
_TM2 = int(os.environ.get('TM2', 128))
_TM3 = int(os.environ.get('TM3', 512))
_PAD = 8
_KC = int(os.environ.get('KC', 256))


def _dft_matrix():
    c = _C
    f = np.concatenate([np.arange(0, c, 2), np.arange(1, c, 2)])
    t = np.arange(c)
    m = ((2 * f[:, None] + 1) * t[None, :]) % (4 * c)
    th = np.pi * m.astype(np.float64) / (2 * c)
    return np.concatenate([np.cos(th), -np.sin(th)], axis=0)


_F_NP = _dft_matrix()


def _ln(x):
    m = jnp.mean(x, axis=-1, keepdims=True)
    xc = x - m
    v = jnp.mean(xc * xc, axis=-1, keepdims=True)
    return xc * jax.lax.rsqrt(v + 1e-5)


def _gelu(x):
    c0 = 0.7978845608028654
    return 0.5 * x * (1.0 + jnp.tanh(c0 * (x + 0.044715 * x * x * x)))


def _silu(x):
    return 0.5 * x * (1.0 + jnp.tanh(0.5 * x))


def _pack(x):
    return pltpu.bitcast(x, jnp.uint32)


def _unpack(x):
    return pltpu.bitcast(x, jnp.bfloat16)


def _kernel(x_hbm, k_hbm, v_hbm, shk_hbm, h_hbm, d_hbm, win_hbm, wsp_hbm, b_hbm, wout_hbm, f_hbm, g_hbm,
            o_hbm,
            x_v, k_v, v_v, shk_v, h_v, d_v, win_v, wsp_v, b_v, wout_v, f_v, g_v,
            xn_s, kv_s, z1_s, z2_s, u_s, hh_s, y_s, o_s, p_s, bcol_s,
            sem_t, sem_m, sem_o, sem_w,
            *, S, D, FH):
    C, TM1, TM2, TM3, KC = _C, _TM1, _TM2, _TM3, _KC
    NT1, NT2, NT3 = S // TM1, S // TM2, S // TM3
    NB = S // C
    f32, bf16 = jnp.float32, jnp.bfloat16

    def rows(i, n):
        if isinstance(i, int):
            return pl.ds(i * n, n)
        return pl.ds(pl.multiple_of(i * n, n), n)

    def put(ref, b, val):
        ref[b, 0:C, :] = val[:C]
        ref[b, C + _PAD:2 * C + _PAD, :] = val[C:]

    def tile_copies(i):
        r = rows(i, TM1)
        return [
            None,
            pltpu.make_async_copy(k_hbm.at[r], k_v.at[pl.ds(pl.multiple_of(i * TM1 + 16, 16), TM1)], sem_t.at[1, i]),
            pltpu.make_async_copy(v_hbm.at[r], v_v.at[r], sem_t.at[2, i]),
            pltpu.make_async_copy(h_hbm.at[:, r], h_v.at[:, r], sem_t.at[3, i]),
        ]

    def wsp_copy(i):
        r = rows(i, TM1)
        return pltpu.make_async_copy(wsp_hbm.at[r], wsp_v.at[r], sem_t.at[4, i])

    misc = [
        None,
        pltpu.make_async_copy(shk_hbm, shk_v, sem_m.at[1]),
        pltpu.make_async_copy(f_hbm, f_v, sem_m.at[2]),
        pltpu.make_async_copy(d_hbm, d_v, sem_m.at[3]),
        pltpu.make_async_copy(b_hbm, b_v, sem_m.at[4]),
        pltpu.make_async_copy(wout_hbm, wout_v, sem_m.at[5]),
        pltpu.make_async_copy(g_hbm, g_v, sem_m.at[6]),
    ]

    x_copy = lambda i: pltpu.make_async_copy(x_hbm.at[rows(i, TM1)], x_v.at[rows(i, TM1)], sem_t.at[0, i])
    kvh_copies = lambda i: tile_copies(i)[1:]
    def win_copy(c):
        c0 = (1 - c) * FH
        return pltpu.make_async_copy(win_hbm.at[:, pl.ds(c0, FH)], win_v.at[:, pl.ds(c0, FH)], sem_w.at[c])

    def once(fn):
        jax.lax.fori_loop(0, 1, lambda i, c: (fn(), c)[1], 0)

    x_copy(0).start()
    win_copy(0).start()
    k_v[pl.ds(0, 16), :] = jnp.zeros((16, D), bf16)
    with jax.named_scope("p0"):
        x_copy(0).wait()
    win_copy(1).start()
    xn_s[rows(0, TM1 // 2), :] = _pack(_ln(x_v[rows(0, TM1), :].astype(f32)).astype(bf16))
    win_copy(0).wait()
    misc[1].start()
    misc[2].start()
    for c in kvh_copies(0):
        c.start()
    x_copy(1).start()

    def first_a():
        xn = _unpack(xn_s[rows(0, TM1 // 2), :])
        z2 = _gelu(jnp.dot(xn, win_v[:, FH:], preferred_element_type=f32))
        z2_s[rows(0, TM1 // 2), :] = _pack(_ln(z2).astype(bf16))

    with jax.named_scope("p0b"):
        once(first_a)
    win_copy(1).wait()
    for c in misc[3:]:
        c.start()

    def first_b():
        xn = _unpack(xn_s[rows(0, TM1 // 2), :])
        z1_s[rows(0, TM1 // 2), :] = _pack(_gelu(jnp.dot(xn, win_v[:, :FH], preferred_element_type=f32)).astype(bf16))

    with jax.named_scope("p0c"):
        once(first_b)
    misc[1].wait()
    misc[2].wait()

    def p1(i, carry, first=False):
        def nxt():
            for c in kvh_copies(i + 1):
                c.start()
            x_copy(i + 1).wait()

        if first:
            nxt()
            x_copy(2).start()
        else:
            pl.when(i + 1 < NT1)(nxt)
            pl.when(i + 2 < NT1)(lambda: x_copy(i + 2).start())

        wsp_copy(i).start()
        for c in kvh_copies(i):
            c.wait()
        r = rows(i, TM1)
        rh = rows(i, TM1 // 2)
        r0 = i * TM1 if first else pl.multiple_of(i * TM1, TM1)
        never = jax.lax.broadcasted_iota(jnp.int32, (8, 128), 0) > (i + 8)

        def anchor(val, d):
            a0 = jnp.where(never, d[0:8, 0:128].astype(val.dtype), val[0:8, 0:128])
            top = jnp.concatenate([a0, val[8:, 0:128]], axis=0)
            return top if val.shape[1] == 128 else jnp.concatenate([top, val[:, 128:]], axis=1)

        never16 = jax.lax.broadcasted_iota(jnp.int32, (16, 128), 0) > (i + 16)
        pins = {}

        def pinned(lhs, j):
            if j not in pins or first:
                return lhs
            t = None
            for pv in pins[j]:
                for c0 in range(0, pv.shape[1], 128):
                    for rr0 in range(0, pv.shape[0], 8 * PST):
                        q = pv[rr0:rr0 + 8, c0:c0 + 128]
                        t = q if t is None else jnp.maximum(t, q)
            t = jnp.concatenate([t, t], axis=0).astype(bf16)
            cols = []
            for c0 in range(0, lhs.shape[1], 128):
                a0 = jnp.where(never16, t, lhs[0:16, c0:c0 + 128])
                cols.append(jnp.concatenate([a0, lhs[16:, c0:c0 + 128]], axis=0))
            return cols[0] if len(cols) == 1 else jnp.concatenate(cols, axis=1)

        PST = int(os.environ.get('PST', 1))
        PL = int(os.environ.get('PL', 4))
        NZ = FH // 128
        BPT = TM1 // C
        fm = f_v[...]
        xn = _unpack(xn_s[rh, :])
        shk = shk_v[...].astype(f32)
        j = 0
        z2 = []
        kvs = []
        KVP = eval(os.environ.get('KVP', '[3,3,5,12,13]'))

        def do_kv(n, anc):
            ls = slice(n * 128, (n + 1) * 128)
            kk = k_v[pl.ds(r0, TM1 + 16), ls].astype(f32)
            if anc is not None:
                kk = anchor(kk, anc)
            ks = kk[16:16 + TM1] * shk[0:1, ls]
            for t in range(1, 4):
                ks = ks + kk[16 - t:16 - t + TM1] * shk[t:t + 1, ls]
            kvn = ks * v_v[r, ls].astype(f32)
            pins.setdefault(KVP[n], []).append(kvn)
            kvn = kvn.astype(bf16)
            kv_s[rh, ls] = _pack(kvn)
            kvs.append(kvn)

        def do_h(bb):
            hb = h_v[:, rows(i * BPT + bb, C)]
            put(hh_s, i * BPT + bb, jax.lax.dot_general(pinned(fm, j), hb, (((1,), (1,)), ((), ())),
                                                        preferred_element_type=f32))

        do_h(0)
        j += 1
        do_kv(0, None)
        do_kv(1, None)
        if first:
            for n in range(2, D // 128):
                do_kv(n, None)
        for n in range(0 if first else NZ):
            d = jnp.dot(pinned(xn, j), win_v[:, FH + n * 128:FH + (n + 1) * 128], preferred_element_type=f32)
            gl = _gelu(d)
            z2.append(gl)
            pins.setdefault(j + PL, []).append(gl)
            if n == 1:
                do_kv(2, d)
            j += 1
        do_h(1)
        j += 1
        if first:
            xx = _ln(x_v[rows(1, TM1), :].astype(f32))
            xn_s[rows(1, TM1 // 2), :] = _pack(xx.astype(bf16))
        else:
            zl = _ln(jnp.concatenate(z2, axis=1))
            z2_s[rh, :] = _pack(zl.astype(bf16))
            pins.setdefault(j + 3, []).append(zl)
        for n in range(0 if first else NZ):
            d = jnp.dot(pinned(xn, j), win_v[:, n * 128:(n + 1) * 128], preferred_element_type=f32)
            gl = _gelu(d)
            z1_s[rh, n * 128:(n + 1) * 128] = _pack(gl.astype(bf16))
            pins.setdefault(j + PL, []).append(gl)
            if n == 1:
                do_kv(3, d)
            if n == 2:
                do_kv(4, d)
            if n == 4:
                inx = jnp.minimum(i + 1, NT1 - 1)
                xx = _ln(anchor(x_v[rows(inx, TM1), :].astype(f32), d))
                xn_s[rows(inx, TM1 // 2), :] = _pack(xx.astype(bf16))
            j += 1
        kv = jnp.concatenate(kvs, axis=1)
        for bb in range(BPT):
            b = i * BPT + bb
            put(u_s, b, jnp.dot(pinned(fm, j), kv[bb * C:(bb + 1) * C, :], preferred_element_type=f32))
            j += 1
        return carry

    with jax.named_scope('p1'):
        with jax.named_scope('p1a'):
            p1(0, 0, first=True)
        jax.lax.fori_loop(1, NT1, p1, 0)
    with jax.named_scope('p1b'):
        for c in misc[3:]:
            c.wait()
        for i in range(NT1):
            wsp_copy(i).wait()

    bcol_s[...] = jnp.broadcast_to(b_v[...].astype(f32).reshape(1, S), (128, S)).T

    NLT = D // 128
    FPS = C // NT2
    dep = []
    last = [None]
    PINW = int(os.environ.get('PINW', 128))
    LAG = int(os.environ.get('LAG', 3))

    def conv_gen(fr0, never):
        sgn = jnp.where(fr0 < C // 2, 1.0, -1.0).astype(f32)
        for c in range(NLT):
            ls = slice(c * 128, (c + 1) * 128)
            for half in range(FPS // 8):
                fre = pl.ds(pl.multiple_of(fr0 + half * 8, 8), 8)
                fim = pl.ds(pl.multiple_of(fr0 + half * 8 + C + _PAD, 8), 8)
                fimy = pl.ds(pl.multiple_of(fr0 + half * 8 + C, 8), 8)
                prev = None
                for b in range(NB):
                    ar = ai = None
                    for m in range(b + 1):
                        hr = hh_s[m, fre, ls]
                        if dep:
                            hr = jnp.where(never, dep.pop(), hr)
                        hi = hh_s[m, fim, ls]
                        ur = u_s[b - m, fre, ls]
                        ui = u_s[b - m, fim, ls]
                        pr = hr * ur - hi * ui
                        pi = hr * ui + hi * ur
                        ar = pr if ar is None else ar + pr
                        ai = pi if ai is None else ai + pi
                        last[0] = ar
                        yield
                    if prev is None:
                        yr, yi = ar, ai
                    else:
                        yr = ar - sgn * prev[1]
                        yi = ai + sgn * prev[0]
                    prev = (ar, ai)
                    y_s[b, fre, ls] = yr
                    y_s[b, fimy, ls] = yi
                    last[0] = yr

    NPAIR = NLT * (FPS // 8) * (NB * (NB + 1) // 2)

    def p2(i, carry):
        r = rows(i, TM2)
        rh = rows(i, TM2 // 2)
        never = jax.lax.broadcasted_iota(jnp.int32, (8, 128), 0) > (i + 8)
        gen = conv_gen(i * FPS, never)
        never16 = jax.lax.broadcasted_iota(jnp.int32, (16, 128), 0) > (i + 16)
        hist = []
        npieces = (FH // 128) * (S // KC)
        per = -(-NPAIR // npieces)

        def pump(d):
            dep.append(d[0:8, 0:128])
            for _ in range(per if not int(os.environ.get('NOCONV', 0)) else 1):
                next(gen, None)
            hist.append(last[0])

        bias = bcol_s[r, :]
        for n in range(FH // 128):
            ns = slice(n * 128, (n + 1) * 128)
            acc = None
            for kc in range(S // KC):
                lhs = wsp_v[r, kc * KC:(kc + 1) * KC]
                if LAG and len(hist) >= LAG:
                    t = jnp.concatenate([hist[-LAG]] * 2, axis=0).astype(bf16)
                    cols = []
                    for c0 in range(0, KC, 128):
                        if c0 < PINW:
                            a0 = jnp.where(never16, t, lhs[0:16, c0:c0 + 128])
                            cols.append(jnp.concatenate([a0, lhs[16:, c0:c0 + 128]], axis=0))
                        else:
                            cols.append(lhs[:, c0:c0 + 128])
                    lhs = cols[0] if len(cols) == 1 else jnp.concatenate(cols, axis=1)
                d = jnp.dot(lhs, _unpack(z2_s[kc * KC // 2:(kc + 1) * KC // 2, ns]),
                            preferred_element_type=f32)
                acc = d if acc is None else acc + d
                pump(d)
            p_s[rh, ns] = _pack((_unpack(z1_s[rh, ns]).astype(f32) * (acc + bias)).astype(bf16))
        if not int(os.environ.get('NOCONV', 0)):
            for _ in gen:
                pass
        return carry

    with jax.named_scope('p2'):
        jax.lax.fori_loop(0, NT2, p2, 0)

    def out_copy(i):
        r = rows(i, TM3)
        return pltpu.make_async_copy(o_s.at[r], o_hbm.at[r], sem_o.at[i])

    def p3(i, carry):
        gm = g_v[...]
        dd = d_v[...].astype(f32).reshape(1, D)
        gate = _silu(jnp.dot(_unpack(p_s[rows(i, TM3 // 2), :]), wout_v[...], preferred_element_type=f32))
        for bb in range(TM3 // C):
            b = i * (TM3 // C) + bb
            rr = rows(b, C)
            rrh = rows(b, C // 2)
            y = jnp.dot(gm, y_s[b].astype(bf16), preferred_element_type=f32)
            y = y + _unpack(kv_s[rrh, :]).astype(f32) * dd
            s = _unpack(xn_s[rrh, :]).astype(f32) * y
            o_s[rr, :] = (x_v[rr, :].astype(f32) + s * gate[bb * C:(bb + 1) * C]).astype(bf16)
        out_copy(i).start()
        return carry

    with jax.named_scope('p3'):
        jax.lax.fori_loop(0, NT3, p3, 0)
    with jax.named_scope('p4'):
        for i in range(NT3):
            out_copy(i).wait()


@jax.jit
def pallas_recurrent_scan__ssm_conv_h3__mixer_gmlp__prompt_kernel(
    A_q: jax.Array,
    A_k: jax.Array,
    A_v: jax.Array,
    A_shift_k: jax.Array,
    A_ssm_k: jax.Array,
    A_ssm_D: jax.Array,
    B_x: jax.Array,
    B_w_in: jax.Array,
    B_w_sp: jax.Array,
    B_b_sp: jax.Array,
    B_w_out: jax.Array,
):
    del B_x
    _, S, D = A_q.shape
    F = B_w_in.shape[-1]
    FH = F // 2
    C = _C
    NB = S // C
    bf16, f32, u32 = jnp.bfloat16, jnp.float32, jnp.uint32

    x = A_q.reshape(S, D)
    k = A_k.reshape(S, D)
    v = A_v.reshape(S, D)
    shk = A_shift_k.T
    dvec = A_ssm_D
    bvec = B_b_sp
    fmat = np.asarray(_F_NP, dtype=np.float32).astype(bf16)
    gmat = np.asarray(_F_NP.T / C, dtype=np.float32).astype(bf16)

    kern = functools.partial(_kernel, S=S, D=D, FH=FH)
    any_spec = pl.BlockSpec(memory_space=pl.ANY)
    out = pl.pallas_call(
        kern,
        out_shape=jax.ShapeDtypeStruct((S, D), bf16),
        in_specs=[any_spec] * 12,
        out_specs=any_spec,
        scratch_shapes=[
            pltpu.VMEM((S, D), bf16),
            pltpu.VMEM((S + 16, D), bf16),
            pltpu.VMEM((S, D), bf16),
            pltpu.VMEM(shk.shape, bf16),
            pltpu.VMEM((D, S), bf16),
            pltpu.VMEM((D,), bf16),
            pltpu.VMEM((D, F), bf16),
            pltpu.VMEM((S, S), bf16),
            pltpu.VMEM((S,), bf16),
            pltpu.VMEM((FH, D), bf16),
            pltpu.VMEM((2 * C, C), bf16),
            pltpu.VMEM((C, 2 * C), bf16),
            pltpu.VMEM((S // 2, D), u32),
            pltpu.VMEM((S // 2, D), u32),
            pltpu.VMEM((S // 2, FH), u32),
            pltpu.VMEM((S // 2, FH), u32),
            pltpu.VMEM((NB, 2 * C + 2 * _PAD, D), f32),
            pltpu.VMEM((NB, 2 * C + 2 * _PAD, D), f32),
            pltpu.VMEM((NB, 2 * C, D), f32),
            pltpu.VMEM((S, D), bf16),
            pltpu.VMEM((S // 2, FH), u32),
            pltpu.VMEM((S, 128), f32),
            pltpu.SemaphoreType.DMA((5, S // _TM1)),
            pltpu.SemaphoreType.DMA((7,)),
            pltpu.SemaphoreType.DMA((S // _TM3,)),
            pltpu.SemaphoreType.DMA((2,)),
        ],
        compiler_params=pltpu.CompilerParams(vmem_limit_bytes=120 * 1024 * 1024),
    )(x, k, v, shk, A_ssm_k, dvec, B_w_in, B_w_sp, bvec, B_w_out, fmat, gmat)
    return out.reshape(1, S, D)
```

```python
import functools
import os

import jax
import jax.numpy as jnp
import numpy as np
import jax.experimental.pallas as pl
import jax.experimental.pallas.tpu as pltpu

_C = 128
_TM1 = int(os.environ.get('TM1', 256))
_TM2 = int(os.environ.get('TM2', 128))
_TM3 = int(os.environ.get('TM3', 512))
_PAD = 8
_KC = int(os.environ.get('KC', 256))


def _dft_matrix():
    c = _C
    f = np.concatenate([np.arange(0, c, 2), np.arange(1, c, 2)])
    t = np.arange(c)
    m = ((2 * f[:, None] + 1) * t[None, :]) % (4 * c)
    th = np.pi * m.astype(np.float64) / (2 * c)
    return np.concatenate([np.cos(th), -np.sin(th)], axis=0)


_F_NP = _dft_matrix()


def _ln(x):
    m = jnp.mean(x, axis=-1, keepdims=True)
    xc = x - m
    v = jnp.mean(xc * xc, axis=-1, keepdims=True)
    return xc * jax.lax.rsqrt(v + 1e-5)


def _gelu(x):
    c0 = 0.7978845608028654
    return 0.5 * x * (1.0 + jnp.tanh(c0 * (x + 0.044715 * x * x * x)))


def _silu(x):
    return 0.5 * x * (1.0 + jnp.tanh(0.5 * x))


def _pack(x):
    return pltpu.bitcast(x, jnp.uint32)


def _unpack(x):
    return pltpu.bitcast(x, jnp.bfloat16)


def _kernel(x_hbm, k_hbm, v_hbm, shk_hbm, h_hbm, d_hbm, win_hbm, wsp_hbm, b_hbm, wout_hbm, f_hbm, g_hbm,
            o_hbm,
            x_v, k_v, v_v, shk_v, h_v, d_v, win_v, wsp_v, b_v, wout_v, f_v, g_v,
            xn_s, kv_s, z1_s, z2_s, u_s, hh_s, y_s, o_s, p_s, bcol_s,
            sem_t, sem_m, sem_o, sem_w,
            *, S, D, FH):
    C, TM1, TM2, TM3, KC = _C, _TM1, _TM2, _TM3, _KC
    NT1, NT2, NT3 = S // TM1, S // TM2, S // TM3
    NB = S // C
    f32, bf16 = jnp.float32, jnp.bfloat16

    def rows(i, n):
        if isinstance(i, int):
            return pl.ds(i * n, n)
        return pl.ds(pl.multiple_of(i * n, n), n)

    def put(ref, b, val):
        ref[b, 0:C, :] = val[:C]
        ref[b, C + _PAD:2 * C + _PAD, :] = val[C:]

    def tile_copies(i):
        r = rows(i, TM1)
        return [
            None,
            pltpu.make_async_copy(k_hbm.at[r], k_v.at[pl.ds(pl.multiple_of(i * TM1 + 16, 16), TM1)], sem_t.at[1, i]),
            pltpu.make_async_copy(v_hbm.at[r], v_v.at[r], sem_t.at[2, i]),
            pltpu.make_async_copy(h_hbm.at[:, r], h_v.at[:, r], sem_t.at[3, i]),
        ]

    def wsp_copy(i):
        r = rows(i, TM1)
        return pltpu.make_async_copy(wsp_hbm.at[r], wsp_v.at[r], sem_t.at[4, i])

    misc = [
        None,
        pltpu.make_async_copy(shk_hbm, shk_v, sem_m.at[1]),
        pltpu.make_async_copy(f_hbm, f_v, sem_m.at[2]),
        pltpu.make_async_copy(d_hbm, d_v, sem_m.at[3]),
        pltpu.make_async_copy(b_hbm, b_v, sem_m.at[4]),
        pltpu.make_async_copy(wout_hbm, wout_v, sem_m.at[5]),
        pltpu.make_async_copy(g_hbm, g_v, sem_m.at[6]),
    ]

    x_copy = lambda i: pltpu.make_async_copy(x_hbm.at[rows(i, TM1)], x_v.at[rows(i, TM1)], sem_t.at[0, i])
    kvh_copies = lambda i: tile_copies(i)[1:]
    def win_copy(c):
        c0 = (1 - c) * FH
        return pltpu.make_async_copy(win_hbm.at[:, pl.ds(c0, FH)], win_v.at[:, pl.ds(c0, FH)], sem_w.at[c])

    def once(fn):
        jax.lax.fori_loop(0, 1, lambda i, c: (fn(), c)[1], 0)

    x_copy(0).start()
    win_copy(0).start()
    k_v[pl.ds(0, 16), :] = jnp.zeros((16, D), bf16)
    with jax.named_scope("p0"):
        x_copy(0).wait()
    win_copy(1).start()
    xn_s[rows(0, TM1 // 2), :] = _pack(_ln(x_v[rows(0, TM1), :].astype(f32)).astype(bf16))
    win_copy(0).wait()
    misc[1].start()
    misc[2].start()
    for c in kvh_copies(0):
        c.start()
    x_copy(1).start()

    def first_a():
        xn = _unpack(xn_s[rows(0, TM1 // 2), :])
        z2 = _gelu(jnp.dot(xn, win_v[:, FH:], preferred_element_type=f32))
        z2_s[rows(0, TM1 // 2), :] = _pack(_ln(z2).astype(bf16))

    with jax.named_scope("p0b"):
        once(first_a)
    win_copy(1).wait()
    for c in misc[3:]:
        c.start()

    def first_b():
        xn = _unpack(xn_s[rows(0, TM1 // 2), :])
        z1_s[rows(0, TM1 // 2), :] = _pack(_gelu(jnp.dot(xn, win_v[:, :FH], preferred_element_type=f32)).astype(bf16))

    with jax.named_scope("p0c"):
        once(first_b)
    misc[1].wait()
    misc[2].wait()

    def p1(i, carry, first=False):
        def nxt():
            for c in kvh_copies(i + 1):
                c.start()
            x_copy(i + 1).wait()

        if first:
            nxt()
            x_copy(2).start()
        else:
            pl.when(i + 1 < NT1)(nxt)
            pl.when(i + 2 < NT1)(lambda: x_copy(i + 2).start())

        wsp_copy(i).start()
        for c in kvh_copies(i):
            c.wait()
        r = rows(i, TM1)
        rh = rows(i, TM1 // 2)
        r0 = i * TM1 if first else pl.multiple_of(i * TM1, TM1)
        never = jax.lax.broadcasted_iota(jnp.int32, (8, 128), 0) > (i + 8)

        def anchor(val, d):
            a0 = jnp.where(never, d[0:8, 0:128].astype(val.dtype), val[0:8, 0:128])
            top = jnp.concatenate([a0, val[8:, 0:128]], axis=0)
            return top if val.shape[1] == 128 else jnp.concatenate([top, val[:, 128:]], axis=1)

        never16 = jax.lax.broadcasted_iota(jnp.int32, (16, 128), 0) > (i + 16)
        pins = {}

        def pinned(lhs, j):
            if j not in pins or first:
                return lhs
            t = None
            for pv in pins[j]:
                for c0 in range(0, pv.shape[1], 128):
                    for rr0 in range(0, pv.shape[0], 8 * PST):
                        q = pv[rr0:rr0 + 8, c0:c0 + 128]
                        t = q if t is None else jnp.maximum(t, q)
            t = jnp.concatenate([t, t], axis=0).astype(bf16)
            cols = []
            for c0 in range(0, lhs.shape[1], 128):
                a0 = jnp.where(never16, t, lhs[0:16, c0:c0 + 128])
                cols.append(jnp.concatenate([a0, lhs[16:, c0:c0 + 128]], axis=0))
            return cols[0] if len(cols) == 1 else jnp.concatenate(cols, axis=1)

        PST = int(os.environ.get('PST', 1))
        PL = int(os.environ.get('PL', 4))
        NZ = FH // 128
        BPT = TM1 // C
        fm = f_v[...]
        xn = _unpack(xn_s[rh, :])
        shk = shk_v[...].astype(f32)
        j = 0
        z2 = []
        kvs = []
        KVP = eval(os.environ.get('KVP', '[3,3,5,12,13]'))

        def do_kv(n, anc):
            ls = slice(n * 128, (n + 1) * 128)
            kk = k_v[pl.ds(r0, TM1 + 16), ls].astype(f32)
            if anc is not None:
                kk = anchor(kk, anc)
            ks = kk[16:16 + TM1] * shk[0:1, ls]
            for t in range(1, 4):
                ks = ks + kk[16 - t:16 - t + TM1] * shk[t:t + 1, ls]
            kvn = ks * v_v[r, ls].astype(f32)
            pins.setdefault(KVP[n], []).append(kvn)
            kvn = kvn.astype(bf16)
            kv_s[rh, ls] = _pack(kvn)
            kvs.append(kvn)

        def do_h(bb):
            hb = h_v[:, rows(i * BPT + bb, C)]
            put(hh_s, i * BPT + bb, jax.lax.dot_general(pinned(fm, j), hb, (((1,), (1,)), ((), ())),
                                                        preferred_element_type=f32))

        do_h(0)
        j += 1
        do_kv(0, None)
        do_kv(1, None)
        if first:
            for n in range(2, D // 128):
                do_kv(n, None)
        for n in range(0 if first else NZ):
            d = jnp.dot(pinned(xn, j), win_v[:, FH + n * 128:FH + (n + 1) * 128], preferred_element_type=f32)
            gl = _gelu(d)
            z2.append(gl)
            pins.setdefault(j + PL, []).append(gl)
            if n == 1:
                do_kv(2, d)
            j += 1
        do_h(1)
        j += 1
        if first:
            xx = _ln(x_v[rows(1, TM1), :].astype(f32))
            xn_s[rows(1, TM1 // 2), :] = _pack(xx.astype(bf16))
        else:
            zl = _ln(jnp.concatenate(z2, axis=1))
            z2_s[rh, :] = _pack(zl.astype(bf16))
            pins.setdefault(j + 3, []).append(zl)
        for n in range(0 if first else NZ):
            d = jnp.dot(pinned(xn, j), win_v[:, n * 128:(n + 1) * 128], preferred_element_type=f32)
            gl = _gelu(d)
            z1_s[rh, n * 128:(n + 1) * 128] = _pack(gl.astype(bf16))
            pins.setdefault(j + PL, []).append(gl)
            if n == 1:
                do_kv(3, d)
            if n == 2:
                do_kv(4, d)
            if n == 4:
                inx = jnp.minimum(i + 1, NT1 - 1)
                xx = _ln(anchor(x_v[rows(inx, TM1), :].astype(f32), d))
                xn_s[rows(inx, TM1 // 2), :] = _pack(xx.astype(bf16))
            j += 1
        kv = jnp.concatenate(kvs, axis=1)
        for bb in range(BPT):
            b = i * BPT + bb
            put(u_s, b, jnp.dot(pinned(fm, j), kv[bb * C:(bb + 1) * C, :], preferred_element_type=f32))
            j += 1
        return carry

    with jax.named_scope('p1'):
        with jax.named_scope('p1a'):
            p1(0, 0, first=True)
        jax.lax.fori_loop(1, NT1, p1, 0, unroll=int(os.environ.get('U1', 1)))
    with jax.named_scope('p1b'):
        for c in misc[3:]:
            c.wait()
        for i in range(NT1):
            wsp_copy(i).wait()

    bcol_s[...] = jnp.broadcast_to(b_v[...].astype(f32).reshape(1, S), (128, S)).T

    NLT = D // 128
    FPS = C // NT2
    dep = []
    last = [None]
    PINW = int(os.environ.get('PINW', 128))
    LAG = int(os.environ.get('LAG', 3))

    def conv_gen(fr0, never):
        sgn = jnp.where(fr0 < C // 2, 1.0, -1.0).astype(f32)
        for c in range(NLT):
            ls = slice(c * 128, (c + 1) * 128)
            for half in range(FPS // 8):
                fre = pl.ds(pl.multiple_of(fr0 + half * 8, 8), 8)
                fim = pl.ds(pl.multiple_of(fr0 + half * 8 + C + _PAD, 8), 8)
                fimy = pl.ds(pl.multiple_of(fr0 + half * 8 + C, 8), 8)
                prev = None
                for b in range(NB):
                    ar = ai = None
                    for m in range(b + 1):
                        hr = hh_s[m, fre, ls]
                        if dep:
                            hr = jnp.where(never, dep.pop(), hr)
                        hi = hh_s[m, fim, ls]
                        ur = u_s[b - m, fre, ls]
                        ui = u_s[b - m, fim, ls]
                        pr = hr * ur - hi * ui
                        pi = hr * ui + hi * ur
                        ar = pr if ar is None else ar + pr
                        ai = pi if ai is None else ai + pi
                        last[0] = ar
                        yield
                    if prev is None:
                        yr, yi = ar, ai
                    else:
                        yr = ar - sgn * prev[1]
                        yi = ai + sgn * prev[0]
                    prev = (ar, ai)
                    y_s[b, fre, ls] = yr
                    y_s[b, fimy, ls] = yi
                    last[0] = yr

    NPAIR = NLT * (FPS // 8) * (NB * (NB + 1) // 2)

    def p2(i, carry):
        r = rows(i, TM2)
        rh = rows(i, TM2 // 2)
        never = jax.lax.broadcasted_iota(jnp.int32, (8, 128), 0) > (i + 8)
        gen = conv_gen(i * FPS, never)
        never16 = jax.lax.broadcasted_iota(jnp.int32, (16, 128), 0) > (i + 16)
        hist = []
        npieces = (FH // 128) * (S // KC)
        per = -(-NPAIR // npieces)

        def pump(d):
            dep.append(d[0:8, 0:128])
            for _ in range(per if not int(os.environ.get('NOCONV', 0)) else 1):
                next(gen, None)
            hist.append(last[0])

        bias = bcol_s[r, :]
        for n in range(FH // 128):
            ns = slice(n * 128, (n + 1) * 128)
            acc = None
            for kc in range(S // KC):
                lhs = wsp_v[r, kc * KC:(kc + 1) * KC]
                if LAG and len(hist) >= LAG:
                    t = jnp.concatenate([hist[-LAG]] * 2, axis=0).astype(bf16)
                    cols = []
                    for c0 in range(0, KC, 128):
                        if c0 < PINW:
                            a0 = jnp.where(never16, t, lhs[0:16, c0:c0 + 128])
                            cols.append(jnp.concatenate([a0, lhs[16:, c0:c0 + 128]], axis=0))
                        else:
                            cols.append(lhs[:, c0:c0 + 128])
                    lhs = cols[0] if len(cols) == 1 else jnp.concatenate(cols, axis=1)
                d = jnp.dot(lhs, _unpack(z2_s[kc * KC // 2:(kc + 1) * KC // 2, ns]),
                            preferred_element_type=f32)
                acc = d if acc is None else acc + d
                pump(d)
            p_s[rh, ns] = _pack((_unpack(z1_s[rh, ns]).astype(f32) * (acc + bias)).astype(bf16))
        if not int(os.environ.get('NOCONV', 0)):
            for _ in gen:
                pass
        return carry

    with jax.named_scope('p2'):
        jax.lax.fori_loop(0, NT2, p2, 0, unroll=int(os.environ.get('U2', 4)))

    def out_copy(i):
        r = rows(i, C)
        return pltpu.make_async_copy(o_s.at[r], o_hbm.at[r], sem_o.at[i])

    def p3(i, carry):
        gm = g_v[...]
        dd = d_v[...].astype(f32).reshape(1, D)
        gate = _silu(jnp.dot(_unpack(p_s[rows(i, TM3 // 2), :]), wout_v[...], preferred_element_type=f32))
        for bb in range(TM3 // C):
            b = i * (TM3 // C) + bb
            rr = rows(b, C)
            rrh = rows(b, C // 2)
            y = jnp.dot(gm, y_s[b].astype(bf16), preferred_element_type=f32)
            y = y + _unpack(kv_s[rrh, :]).astype(f32) * dd
            s = _unpack(xn_s[rrh, :]).astype(f32) * y
            o_s[rr, :] = (x_v[rr, :].astype(f32) + s * gate[bb * C:(bb + 1) * C]).astype(bf16)
            out_copy(b).start()
        return carry

    with jax.named_scope('p3'):
        jax.lax.fori_loop(0, NT3, p3, 0, unroll=int(os.environ.get('U3', 4)))
    with jax.named_scope('p4'):
        for i in range(NB):
            out_copy(i).wait()


@jax.jit
def pallas_recurrent_scan__ssm_conv_h3__mixer_gmlp__prompt_kernel(
    A_q: jax.Array,
    A_k: jax.Array,
    A_v: jax.Array,
    A_shift_k: jax.Array,
    A_ssm_k: jax.Array,
    A_ssm_D: jax.Array,
    B_x: jax.Array,
    B_w_in: jax.Array,
    B_w_sp: jax.Array,
    B_b_sp: jax.Array,
    B_w_out: jax.Array,
):
    del B_x
    _, S, D = A_q.shape
    F = B_w_in.shape[-1]
    FH = F // 2
    C = _C
    NB = S // C
    bf16, f32, u32 = jnp.bfloat16, jnp.float32, jnp.uint32

    x = A_q.reshape(S, D)
    k = A_k.reshape(S, D)
    v = A_v.reshape(S, D)
    shk = A_shift_k.T
    dvec = A_ssm_D
    bvec = B_b_sp
    fmat = np.asarray(_F_NP, dtype=np.float32).astype(bf16)
    gmat = np.asarray(_F_NP.T / C, dtype=np.float32).astype(bf16)

    kern = functools.partial(_kernel, S=S, D=D, FH=FH)
    any_spec = pl.BlockSpec(memory_space=pl.ANY)
    out = pl.pallas_call(
        kern,
        out_shape=jax.ShapeDtypeStruct((S, D), bf16),
        in_specs=[any_spec] * 12,
        out_specs=any_spec,
        scratch_shapes=[
            pltpu.VMEM((S, D), bf16),
            pltpu.VMEM((S + 16, D), bf16),
            pltpu.VMEM((S, D), bf16),
            pltpu.VMEM(shk.shape, bf16),
            pltpu.VMEM((D, S), bf16),
            pltpu.VMEM((D,), bf16),
            pltpu.VMEM((D, F), bf16),
            pltpu.VMEM((S, S), bf16),
            pltpu.VMEM((S,), bf16),
            pltpu.VMEM((FH, D), bf16),
            pltpu.VMEM((2 * C, C), bf16),
            pltpu.VMEM((C, 2 * C), bf16),
            pltpu.VMEM((S // 2, D), u32),
            pltpu.VMEM((S // 2, D), u32),
            pltpu.VMEM((S // 2, FH), u32),
            pltpu.VMEM((S // 2, FH), u32),
            pltpu.VMEM((NB, 2 * C + 2 * _PAD, D), f32),
            pltpu.VMEM((NB, 2 * C + 2 * _PAD, D), f32),
            pltpu.VMEM((NB, 2 * C, D), f32),
            pltpu.VMEM((S, D), bf16),
            pltpu.VMEM((S // 2, FH), u32),
            pltpu.VMEM((S, 128), f32),
            pltpu.SemaphoreType.DMA((5, S // _TM1)),
            pltpu.SemaphoreType.DMA((7,)),
            pltpu.SemaphoreType.DMA((NB,)),
            pltpu.SemaphoreType.DMA((2,)),
        ],
        compiler_params=pltpu.CompilerParams(vmem_limit_bytes=120 * 1024 * 1024),
    )(x, k, v, shk, A_ssm_k, dvec, B_w_in, B_w_sp, bvec, B_w_out, fmat, gmat)
    return out.reshape(1, S, D)
```

```python
import functools

import jax
import jax.numpy as jnp
import numpy as np
import jax.experimental.pallas as pl
import jax.experimental.pallas.tpu as pltpu

_C = 128
_TM1 = 256
_TM2 = 128
_TM3 = 512
_PAD = 8
_KC = 256


def _dft_matrix():
    c = _C
    f = np.concatenate([np.arange(0, c, 2), np.arange(1, c, 2)])
    t = np.arange(c)
    m = ((2 * f[:, None] + 1) * t[None, :]) % (4 * c)
    th = np.pi * m.astype(np.float64) / (2 * c)
    return np.concatenate([np.cos(th), -np.sin(th)], axis=0)


_F_NP = _dft_matrix()


def _ln(x):
    m = jnp.mean(x, axis=-1, keepdims=True)
    xc = x - m
    v = jnp.mean(xc * xc, axis=-1, keepdims=True)
    return xc * jax.lax.rsqrt(v + 1e-5)


def _gelu(x):
    c0 = 0.7978845608028654
    return 0.5 * x * (1.0 + jnp.tanh(x * (c0 + (c0 * 0.044715) * (x * x))))


def _silu(x):
    return 0.5 * x * (1.0 + jnp.tanh(0.5 * x))


def _pack(x):
    return pltpu.bitcast(x, jnp.uint32)


def _unpack(x):
    return pltpu.bitcast(x, jnp.bfloat16)


def _kernel(x_hbm, k_hbm, v_hbm, shk_hbm, h_hbm, d_hbm, win_hbm, wsp_hbm, b_hbm, wout_hbm, f_hbm, g_hbm,
            o_hbm,
            x_v, k_v, v_v, shk_v, h_v, d_v, win_v, wsp_v, b_v, wout_v, f_v, g_v,
            xn_s, kv_s, z1_s, z2_s, u_s, hh_s, y_s, o_s, p_s, bcol_s,
            sem_t, sem_m, sem_o, sem_w,
            *, S, D, FH):
    C, TM1, TM2, TM3, KC = _C, _TM1, _TM2, _TM3, _KC
    NT1, NT2, NT3 = S // TM1, S // TM2, S // TM3
    NB = S // C
    f32, bf16 = jnp.float32, jnp.bfloat16

    def rows(i, n):
        if isinstance(i, int):
            return pl.ds(i * n, n)
        return pl.ds(pl.multiple_of(i * n, n), n)

    def put(ref, b, val):
        ref[b, 0:C, :] = val[:C]
        ref[b, C + _PAD:2 * C + _PAD, :] = val[C:]

    def tile_copies(i):
        r = rows(i, TM1)
        return [
            None,
            pltpu.make_async_copy(k_hbm.at[r], k_v.at[pl.ds(pl.multiple_of(i * TM1 + 16, 16), TM1)], sem_t.at[1, i]),
            pltpu.make_async_copy(v_hbm.at[r], v_v.at[r], sem_t.at[2, i]),
            pltpu.make_async_copy(h_hbm.at[:, r], h_v.at[:, r], sem_t.at[3, i]),
        ]

    def wsp_copy(i):
        r = rows(i, TM1)
        return pltpu.make_async_copy(wsp_hbm.at[r], wsp_v.at[r], sem_t.at[4, i])

    misc = [
        None,
        pltpu.make_async_copy(shk_hbm, shk_v, sem_m.at[1]),
        pltpu.make_async_copy(f_hbm, f_v, sem_m.at[2]),
        pltpu.make_async_copy(d_hbm, d_v, sem_m.at[3]),
        pltpu.make_async_copy(b_hbm, b_v, sem_m.at[4]),
        pltpu.make_async_copy(wout_hbm, wout_v, sem_m.at[5]),
        pltpu.make_async_copy(g_hbm, g_v, sem_m.at[6]),
    ]

    x_copy = lambda i: pltpu.make_async_copy(x_hbm.at[rows(i, TM1)], x_v.at[rows(i, TM1)], sem_t.at[0, i])
    kvh_copies = lambda i: tile_copies(i)[1:]
    def win_copy(c):
        c0 = (1 - c) * FH
        return pltpu.make_async_copy(win_hbm.at[:, pl.ds(c0, FH)], win_v.at[:, pl.ds(c0, FH)], sem_w.at[c])

    def once(fn):
        jax.lax.fori_loop(0, 1, lambda i, c: (fn(), c)[1], 0)

    x_copy(0).start()
    win_copy(0).start()
    k_v[pl.ds(0, 16), :] = jnp.zeros((16, D), bf16)
    with jax.named_scope("p0"):
        x_copy(0).wait()
    win_copy(1).start()
    xn_s[rows(0, TM1 // 2), :] = _pack(_ln(x_v[rows(0, TM1), :].astype(f32)).astype(bf16))
    win_copy(0).wait()
    misc[1].start()
    misc[2].start()
    for c in kvh_copies(0):
        c.start()
    x_copy(1).start()

    def first_a():
        xn = _unpack(xn_s[rows(0, TM1 // 2), :])
        z2 = _gelu(jnp.dot(xn, win_v[:, FH:], preferred_element_type=f32))
        z2_s[rows(0, TM1 // 2), :] = _pack(_ln(z2).astype(bf16))

    with jax.named_scope("p0b"):
        once(first_a)
    win_copy(1).wait()
    for c in misc[3:]:
        c.start()

    def first_b():
        xn = _unpack(xn_s[rows(0, TM1 // 2), :])
        z1_s[rows(0, TM1 // 2), :] = _pack(_gelu(jnp.dot(xn, win_v[:, :FH], preferred_element_type=f32)).astype(bf16))

    with jax.named_scope("p0c"):
        once(first_b)
    misc[1].wait()
    misc[2].wait()

    def p1(i, carry, first=False):
        def nxt():
            for c in kvh_copies(i + 1):
                c.start()
            x_copy(i + 1).wait()

        if first:
            nxt()
            x_copy(2).start()
        else:
            pl.when(i + 1 < NT1)(nxt)
            pl.when(i + 2 < NT1)(lambda: x_copy(i + 2).start())

        wsp_copy(i).start()
        for c in kvh_copies(i):
            c.wait()
        r = rows(i, TM1)
        rh = rows(i, TM1 // 2)
        r0 = i * TM1 if first else pl.multiple_of(i * TM1, TM1)
        never = jax.lax.broadcasted_iota(jnp.int32, (8, 128), 0) > (i + 8)

        def anchor(val, d):
            a0 = jnp.where(never, d[0:8, 0:128].astype(val.dtype), val[0:8, 0:128])
            top = jnp.concatenate([a0, val[8:, 0:128]], axis=0)
            return top if val.shape[1] == 128 else jnp.concatenate([top, val[:, 128:]], axis=1)

        never16 = jax.lax.broadcasted_iota(jnp.int32, (16, 128), 0) > (i + 16)
        pins = {}

        def pinned(lhs, j):
            if j not in pins or first:
                return lhs
            t = None
            for pv in pins[j]:
                for c0 in range(0, pv.shape[1], 128):
                    for rr0 in range(0, pv.shape[0], 8 * PST):
                        q = pv[rr0:rr0 + 8, c0:c0 + 128]
                        t = q if t is None else jnp.maximum(t, q)
            t = jnp.concatenate([t, t], axis=0).astype(bf16)
            cols = []
            for c0 in range(0, lhs.shape[1], 128):
                a0 = jnp.where(never16, t, lhs[0:16, c0:c0 + 128])
                cols.append(jnp.concatenate([a0, lhs[16:, c0:c0 + 128]], axis=0))
            return cols[0] if len(cols) == 1 else jnp.concatenate(cols, axis=1)

        PST = 1
        PL = 4
        NZ = FH // 128
        BPT = TM1 // C
        fm = f_v[...]
        xn = _unpack(xn_s[rh, :])
        shk = shk_v[...].astype(f32)
        j = 0
        z2 = []
        kvs = []
        KVP = [3, 3, 5, 12, 13]

        def do_kv(n, anc):
            ls = slice(n * 128, (n + 1) * 128)
            kk = k_v[pl.ds(r0, TM1 + 16), ls].astype(f32)
            if anc is not None:
                kk = anchor(kk, anc)
            ks = kk[16:16 + TM1] * shk[0:1, ls]
            for t in range(1, 4):
                ks = ks + kk[16 - t:16 - t + TM1] * shk[t:t + 1, ls]
            kvn = ks * v_v[r, ls].astype(f32)
            pins.setdefault(KVP[n], []).append(kvn)
            kvn = kvn.astype(bf16)
            kv_s[rh, ls] = _pack(kvn)
            kvs.append(kvn)

        def do_h(bb):
            hb = h_v[:, rows(i * BPT + bb, C)]
            put(hh_s, i * BPT + bb, jax.lax.dot_general(pinned(fm, j), hb, (((1,), (1,)), ((), ())),
                                                        preferred_element_type=f32))

        do_h(0)
        j += 1
        do_kv(0, None)
        do_kv(1, None)
        if first:
            for n in range(2, D // 128):
                do_kv(n, None)
        for n in range(0 if first else NZ):
            d = jnp.dot(pinned(xn, j), win_v[:, FH + n * 128:FH + (n + 1) * 128], preferred_element_type=f32)
            gl = _gelu(d)
            z2.append(gl)
            pins.setdefault(j + PL, []).append(gl)
            if n == 1:
                do_kv(2, d)
            j += 1
        do_h(1)
        j += 1
        if first:
            xx = _ln(x_v[rows(1, TM1), :].astype(f32))
            xn_s[rows(1, TM1 // 2), :] = _pack(xx.astype(bf16))
        else:
            zl = _ln(jnp.concatenate(z2, axis=1))
            z2_s[rh, :] = _pack(zl.astype(bf16))
            pins.setdefault(j + 3, []).append(zl)
        for n in range(0 if first else NZ):
            d = jnp.dot(pinned(xn, j), win_v[:, n * 128:(n + 1) * 128], preferred_element_type=f32)
            gl = _gelu(d)
            z1_s[rh, n * 128:(n + 1) * 128] = _pack(gl.astype(bf16))
            pins.setdefault(j + PL, []).append(gl)
            if n == 1:
                do_kv(3, d)
            if n == 2:
                do_kv(4, d)
            if n == 4:
                inx = jnp.minimum(i + 1, NT1 - 1)
                xx = _ln(anchor(x_v[rows(inx, TM1), :].astype(f32), d))
                xn_s[rows(inx, TM1 // 2), :] = _pack(xx.astype(bf16))
            j += 1
        kv = jnp.concatenate(kvs, axis=1)
        for bb in range(BPT):
            b = i * BPT + bb
            put(u_s, b, jnp.dot(pinned(fm, j), kv[bb * C:(bb + 1) * C, :], preferred_element_type=f32))
            j += 1
        return carry

    with jax.named_scope('p1'):
        with jax.named_scope('p1a'):
            p1(0, 0, first=True)
        jax.lax.fori_loop(1, NT1, p1, 0, unroll=1)
    with jax.named_scope('p1b'):
        for c in misc[3:]:
            c.wait()
        for i in range(NT1):
            wsp_copy(i).wait()

    bcol_s[...] = jnp.broadcast_to(b_v[...].astype(f32).reshape(1, S), (128, S)).T

    NLT = D // 128
    FPS = C // NT2
    dep = []
    last = [None]
    PINW = 128
    LAG = 3

    def conv_gen(fr0, never):
        sgn = jnp.where(fr0 < C // 2, 1.0, -1.0).astype(f32)
        for c in range(NLT):
            ls = slice(c * 128, (c + 1) * 128)
            for half in range(FPS // 8):
                fre = pl.ds(pl.multiple_of(fr0 + half * 8, 8), 8)
                fim = pl.ds(pl.multiple_of(fr0 + half * 8 + C + _PAD, 8), 8)
                fimy = pl.ds(pl.multiple_of(fr0 + half * 8 + C, 8), 8)
                prev = None
                for b in range(NB):
                    ar = ai = None
                    for m in range(b + 1):
                        hr = hh_s[m, fre, ls]
                        if dep:
                            hr = jnp.where(never, dep.pop(), hr)
                        hi = hh_s[m, fim, ls]
                        ur = u_s[b - m, fre, ls]
                        ui = u_s[b - m, fim, ls]
                        pr = hr * ur - hi * ui
                        pi = hr * ui + hi * ur
                        ar = pr if ar is None else ar + pr
                        ai = pi if ai is None else ai + pi
                        last[0] = ar
                        yield
                    if prev is None:
                        yr, yi = ar, ai
                    else:
                        yr = ar - sgn * prev[1]
                        yi = ai + sgn * prev[0]
                    prev = (ar, ai)
                    y_s[b, fre, ls] = yr
                    y_s[b, fimy, ls] = yi
                    last[0] = yr

    NPAIR = NLT * (FPS // 8) * (NB * (NB + 1) // 2)

    def p2(i, carry):
        r = rows(i, TM2)
        rh = rows(i, TM2 // 2)
        never = jax.lax.broadcasted_iota(jnp.int32, (8, 128), 0) > (i + 8)
        gen = conv_gen(i * FPS, never)
        never16 = jax.lax.broadcasted_iota(jnp.int32, (16, 128), 0) > (i + 16)
        hist = []
        npieces = (FH // 128) * (S // KC)
        per = -(-NPAIR // npieces)

        def pump(d):
            dep.append(d[0:8, 0:128])
            for _ in range(per):
                next(gen, None)
            hist.append(last[0])

        bias = bcol_s[r, :]
        for n in range(FH // 128):
            ns = slice(n * 128, (n + 1) * 128)
            acc = None
            for kc in range(S // KC):
                lhs = wsp_v[r, kc * KC:(kc + 1) * KC]
                if LAG and len(hist) >= LAG:
                    t = jnp.concatenate([hist[-LAG]] * 2, axis=0).astype(bf16)
                    cols = []
                    for c0 in range(0, KC, 128):
                        if c0 < PINW:
                            a0 = jnp.where(never16, t, lhs[0:16, c0:c0 + 128])
                            cols.append(jnp.concatenate([a0, lhs[16:, c0:c0 + 128]], axis=0))
                        else:
                            cols.append(lhs[:, c0:c0 + 128])
                    lhs = cols[0] if len(cols) == 1 else jnp.concatenate(cols, axis=1)
                d = jnp.dot(lhs, _unpack(z2_s[kc * KC // 2:(kc + 1) * KC // 2, ns]),
                            preferred_element_type=f32)
                acc = d if acc is None else acc + d
                pump(d)
            p_s[rh, ns] = _pack((_unpack(z1_s[rh, ns]).astype(f32) * (acc + bias)).astype(bf16))
        for _ in gen:
            pass
        return carry

    with jax.named_scope('p2'):
        jax.lax.fori_loop(0, NT2, p2, 0, unroll=4)

    def out_copy(i):
        r = rows(i, C)
        return pltpu.make_async_copy(o_s.at[r], o_hbm.at[r], sem_o.at[i])

    def p3(i, carry):
        gm = g_v[...]
        dd = d_v[...].astype(f32).reshape(1, D)
        gate = _silu(jnp.dot(_unpack(p_s[rows(i, TM3 // 2), :]), wout_v[...], preferred_element_type=f32))
        for bb in range(TM3 // C):
            b = i * (TM3 // C) + bb
            rr = rows(b, C)
            rrh = rows(b, C // 2)
            y = jnp.dot(gm, y_s[b].astype(bf16), preferred_element_type=f32)
            y = y + _unpack(kv_s[rrh, :]).astype(f32) * dd
            s = _unpack(xn_s[rrh, :]).astype(f32) * y
            o_s[rr, :] = (x_v[rr, :].astype(f32) + s * gate[bb * C:(bb + 1) * C]).astype(bf16)
            out_copy(b).start()
        return carry

    with jax.named_scope('p3'):
        jax.lax.fori_loop(0, NT3, p3, 0, unroll=4)
    with jax.named_scope('p4'):
        for i in range(NB):
            out_copy(i).wait()


@jax.jit
def pallas_recurrent_scan__ssm_conv_h3__mixer_gmlp__prompt_kernel(
    A_q: jax.Array,
    A_k: jax.Array,
    A_v: jax.Array,
    A_shift_k: jax.Array,
    A_ssm_k: jax.Array,
    A_ssm_D: jax.Array,
    B_x: jax.Array,
    B_w_in: jax.Array,
    B_w_sp: jax.Array,
    B_b_sp: jax.Array,
    B_w_out: jax.Array,
):
    del B_x
    _, S, D = A_q.shape
    F = B_w_in.shape[-1]
    FH = F // 2
    C = _C
    NB = S // C
    bf16, f32, u32 = jnp.bfloat16, jnp.float32, jnp.uint32

    x = A_q.reshape(S, D)
    k = A_k.reshape(S, D)
    v = A_v.reshape(S, D)
    shk = A_shift_k.T
    dvec = A_ssm_D
    bvec = B_b_sp
    fmat = np.asarray(_F_NP, dtype=np.float32).astype(bf16)
    gmat = np.asarray(_F_NP.T / C, dtype=np.float32).astype(bf16)

    kern = functools.partial(_kernel, S=S, D=D, FH=FH)
    any_spec = pl.BlockSpec(memory_space=pl.ANY)
    out = pl.pallas_call(
        kern,
        out_shape=jax.ShapeDtypeStruct((S, D), bf16),
        in_specs=[any_spec] * 12,
        out_specs=any_spec,
        scratch_shapes=[
            pltpu.VMEM((S, D), bf16),
            pltpu.VMEM((S + 16, D), bf16),
            pltpu.VMEM((S, D), bf16),
            pltpu.VMEM(shk.shape, bf16),
            pltpu.VMEM((D, S), bf16),
            pltpu.VMEM((D,), bf16),
            pltpu.VMEM((D, F), bf16),
            pltpu.VMEM((S, S), bf16),
            pltpu.VMEM((S,), bf16),
            pltpu.VMEM((FH, D), bf16),
            pltpu.VMEM((2 * C, C), bf16),
            pltpu.VMEM((C, 2 * C), bf16),
            pltpu.VMEM((S // 2, D), u32),
            pltpu.VMEM((S // 2, D), u32),
            pltpu.VMEM((S // 2, FH), u32),
            pltpu.VMEM((S // 2, FH), u32),
            pltpu.VMEM((NB, 2 * C + 2 * _PAD, D), f32),
            pltpu.VMEM((NB, 2 * C + 2 * _PAD, D), f32),
            pltpu.VMEM((NB, 2 * C, D), f32),
            pltpu.VMEM((S, D), bf16),
            pltpu.VMEM((S // 2, FH), u32),
            pltpu.VMEM((S, 128), f32),
            pltpu.SemaphoreType.DMA((5, S // _TM1)),
            pltpu.SemaphoreType.DMA((7,)),
            pltpu.SemaphoreType.DMA((NB,)),
            pltpu.SemaphoreType.DMA((2,)),
        ],
        compiler_params=pltpu.CompilerParams(vmem_limit_bytes=120 * 1024 * 1024),
    )(x, k, v, shk, A_ssm_k, dvec, B_w_in, B_w_sp, bvec, B_w_out, fmat, gmat)
    return out.reshape(1, S, D)
```

```python
import functools

import jax
import jax.numpy as jnp
import numpy as np
import jax.experimental.pallas as pl
import jax.experimental.pallas.tpu as pltpu

_C = 128
_TM1 = 256
_TM2 = 128
_TM3 = 512
_PAD = 8
_KC = 256


def _dft_matrix():
    c = _C
    f = np.concatenate([np.arange(0, c, 2), np.arange(1, c, 2)])
    t = np.arange(c)
    m = ((2 * f[:, None] + 1) * t[None, :]) % (4 * c)
    th = np.pi * m.astype(np.float64) / (2 * c)
    sg = np.where(f % 2 == 0, 1.0, -1.0)[:, None]
    return np.concatenate([np.cos(th), -sg * np.sin(th)], axis=0)


_F_NP = _dft_matrix()


def _ln(x):
    m = jnp.mean(x, axis=-1, keepdims=True)
    xc = x - m
    v = jnp.mean(xc * xc, axis=-1, keepdims=True)
    return xc * jax.lax.rsqrt(v + 1e-5)


def _gelu(x):
    c0 = 0.7978845608028654
    return 0.5 * x * (1.0 + jnp.tanh(x * (c0 + (c0 * 0.044715) * (x * x))))


def _silu(x):
    return 0.5 * x * (1.0 + jnp.tanh(0.5 * x))


def _pack(x):
    return pltpu.bitcast(x, jnp.uint32)


def _unpack(x):
    return pltpu.bitcast(x, jnp.bfloat16)


def _kernel(x_hbm, k_hbm, v_hbm, shk_hbm, h_hbm, d_hbm, win_hbm, wsp_hbm, b_hbm, wout_hbm, f_hbm, g_hbm,
            o_hbm,
            x_v, k_v, v_v, shk_v, h_v, d_v, win_v, wsp_v, b_v, wout_v, f_v, g_v,
            xn_s, kv_s, z1_s, z2_s, u_s, hh_s, y_s, o_s, p_s, bcol_s, kf_s,
            sem_t, sem_m, sem_o, sem_w,
            *, S, D, FH):
    C, TM1, TM2, TM3, KC = _C, _TM1, _TM2, _TM3, _KC
    NT1, NT2, NT3 = S // TM1, S // TM2, S // TM3
    NB = S // C
    f32, bf16 = jnp.float32, jnp.bfloat16

    def rows(i, n):
        if isinstance(i, int):
            return pl.ds(i * n, n)
        return pl.ds(pl.multiple_of(i * n, n), n)

    def put(ref, b, val):
        ref[b, 0:C, :] = val[:C]
        ref[b, C + _PAD:2 * C + _PAD, :] = val[C:]

    def tile_copies(i):
        r = rows(i, TM1)
        return [
            None,
            pltpu.make_async_copy(k_hbm.at[r], k_v.at[pl.ds(pl.multiple_of(i * TM1 + 16, 16), TM1)], sem_t.at[1, i]),
            pltpu.make_async_copy(v_hbm.at[r], v_v.at[r], sem_t.at[2, i]),
            pltpu.make_async_copy(h_hbm.at[:, r], h_v.at[:, r], sem_t.at[3, i]),
        ]

    def wsp_copy(i):
        r = rows(i, TM1)
        return pltpu.make_async_copy(wsp_hbm.at[r], wsp_v.at[r], sem_t.at[4, i])

    misc = [
        None,
        pltpu.make_async_copy(shk_hbm, shk_v, sem_m.at[1]),
        pltpu.make_async_copy(f_hbm, f_v, sem_m.at[2]),
        pltpu.make_async_copy(d_hbm, d_v, sem_m.at[3]),
        pltpu.make_async_copy(b_hbm, b_v, sem_m.at[4]),
        pltpu.make_async_copy(wout_hbm, wout_v, sem_m.at[5]),
        pltpu.make_async_copy(g_hbm, g_v, sem_m.at[6]),
    ]

    x_copy = lambda i: pltpu.make_async_copy(x_hbm.at[rows(i, TM1)], x_v.at[rows(i, TM1)], sem_t.at[0, i])
    kvh_copies = lambda i: tile_copies(i)[1:]
    def win_copy(c):
        c0 = (1 - c) * FH
        return pltpu.make_async_copy(win_hbm.at[:, pl.ds(c0, FH)], win_v.at[:, pl.ds(c0, FH)], sem_w.at[c])

    def once(fn):
        jax.lax.fori_loop(0, 1, lambda i, c: (fn(), c)[1], 0)

    x_copy(0).start()
    win_copy(0).start()
    k_v[pl.ds(0, 16), :] = jnp.zeros((16, D), bf16)
    with jax.named_scope("p0"):
        x_copy(0).wait()
    win_copy(1).start()
    xn_s[rows(0, TM1 // 2), :] = _pack(_ln(x_v[rows(0, TM1), :].astype(f32)).astype(bf16))
    win_copy(0).wait()
    misc[1].start()
    misc[2].start()
    for c in kvh_copies(0):
        c.start()
    x_copy(1).start()

    def first_a():
        xn = _unpack(xn_s[rows(0, TM1 // 2), :])
        z2 = _gelu(jnp.dot(xn, win_v[:, FH:], preferred_element_type=f32))
        z2_s[rows(0, TM1 // 2), :] = _pack(_ln(z2).astype(bf16))

    with jax.named_scope("p0b"):
        once(first_a)
    win_copy(1).wait()
    for c in misc[3:]:
        c.start()

    def first_b():
        xn = _unpack(xn_s[rows(0, TM1 // 2), :])
        z1_s[rows(0, TM1 // 2), :] = _pack(_gelu(jnp.dot(xn, win_v[:, :FH], preferred_element_type=f32)).astype(bf16))

    with jax.named_scope("p0c"):
        once(first_b)
    misc[1].wait()
    misc[2].wait()

    def p1(i, carry, first=False):
        def nxt():
            for c in kvh_copies(i + 1):
                c.start()
            x_copy(i + 1).wait()

        if first:
            nxt()
            x_copy(2).start()
        else:
            pl.when(i + 1 < NT1)(nxt)
            pl.when(i + 2 < NT1)(lambda: x_copy(i + 2).start())

        wsp_copy(i).start()
        for c in kvh_copies(i):
            c.wait()
        r = rows(i, TM1)
        rh = rows(i, TM1 // 2)
        r0 = i * TM1 if first else pl.multiple_of(i * TM1, TM1)
        never = jax.lax.broadcasted_iota(jnp.int32, (8, 128), 0) > (i + 8)

        def anchor(val, d):
            a0 = jnp.where(never, d[0:8, 0:128].astype(val.dtype), val[0:8, 0:128])
            top = jnp.concatenate([a0, val[8:, 0:128]], axis=0)
            return top if val.shape[1] == 128 else jnp.concatenate([top, val[:, 128:]], axis=1)

        never16 = jax.lax.broadcasted_iota(jnp.int32, (16, 128), 0) > (i + 16)
        pins = {}

        def pinned(lhs, j):
            if j not in pins or first:
                return lhs
            t = None
            for pv in pins[j]:
                for c0 in range(0, pv.shape[1], 128):
                    for rr0 in range(0, pv.shape[0], 8 * PST):
                        q = pv[rr0:rr0 + 8, c0:c0 + 128]
                        t = q if t is None else jnp.maximum(t, q)
            t = jnp.concatenate([t, t], axis=0).astype(bf16)
            cols = []
            for c0 in range(0, lhs.shape[1], 128):
                a0 = jnp.where(never16, t, lhs[0:16, c0:c0 + 128])
                cols.append(jnp.concatenate([a0, lhs[16:, c0:c0 + 128]], axis=0))
            return cols[0] if len(cols) == 1 else jnp.concatenate(cols, axis=1)

        PST = 1
        PL = 4
        NZ = FH // 128
        BPT = TM1 // C
        fm = f_v[...]
        xn = _unpack(xn_s[rh, :])
        shk = shk_v[...].astype(f32)
        j = 0
        z2 = []
        kvs = []
        KVP = [3, 3, 5, 12, 13]

        def do_kv(n, anc):
            ls = slice(n * 128, (n + 1) * 128)
            kk = k_v[pl.ds(r0, TM1 + 16), ls].astype(f32)
            if anc is not None:
                kk = anchor(kk, anc)
            kf_s[n] = kk[8:]
            ks = kk[16:16 + TM1] * shk[0:1, ls]
            for t in range(1, 4):
                ks = ks + kf_s[n, 8 - t:8 - t + TM1, :] * shk[t:t + 1, ls]
            kvn = ks * v_v[r, ls].astype(f32)
            pins.setdefault(KVP[n], []).append(kvn)
            kvn = kvn.astype(bf16)
            kv_s[rh, ls] = _pack(kvn)
            kvs.append(kvn)

        def do_h(bb):
            hb = h_v[:, rows(i * BPT + bb, C)]
            put(hh_s, i * BPT + bb, jax.lax.dot_general(pinned(fm, j), hb, (((1,), (1,)), ((), ())),
                                                        preferred_element_type=f32))

        do_h(0)
        j += 1
        do_kv(0, None)
        do_kv(1, None)
        if first:
            for n in range(2, D // 128):
                do_kv(n, None)
        for n in range(0 if first else NZ):
            d = jnp.dot(pinned(xn, j), win_v[:, FH + n * 128:FH + (n + 1) * 128], preferred_element_type=f32)
            gl = _gelu(d)
            z2.append(gl)
            pins.setdefault(j + PL, []).append(gl)
            if n == 1:
                do_kv(2, d)
            j += 1
        do_h(1)
        j += 1
        if first:
            xx = _ln(x_v[rows(1, TM1), :].astype(f32))
            xn_s[rows(1, TM1 // 2), :] = _pack(xx.astype(bf16))
        else:
            zl = _ln(jnp.concatenate(z2, axis=1))
            z2_s[rh, :] = _pack(zl.astype(bf16))
            pins.setdefault(j + 3, []).append(zl)
        for n in range(0 if first else NZ):
            d = jnp.dot(pinned(xn, j), win_v[:, n * 128:(n + 1) * 128], preferred_element_type=f32)
            gl = _gelu(d)
            z1_s[rh, n * 128:(n + 1) * 128] = _pack(gl.astype(bf16))
            pins.setdefault(j + PL, []).append(gl)
            if n == 1:
                do_kv(3, d)
            if n == 2:
                do_kv(4, d)
            if n == 4:
                inx = jnp.minimum(i + 1, NT1 - 1)
                xx = _ln(anchor(x_v[rows(inx, TM1), :].astype(f32), d))
                xn_s[rows(inx, TM1 // 2), :] = _pack(xx.astype(bf16))
            j += 1
        kv = jnp.concatenate(kvs, axis=1)
        for bb in range(BPT):
            b = i * BPT + bb
            put(u_s, b, jnp.dot(pinned(fm, j), kv[bb * C:(bb + 1) * C, :], preferred_element_type=f32))
            j += 1
        return carry

    with jax.named_scope('p1'):
        with jax.named_scope('p1a'):
            p1(0, 0, first=True)
        jax.lax.fori_loop(1, NT1, p1, 0, unroll=1)
    with jax.named_scope('p1b'):
        for c in misc[3:]:
            c.wait()
        for i in range(NT1):
            wsp_copy(i).wait()

    bcol_s[...] = jnp.broadcast_to(b_v[...].astype(f32).reshape(1, S), (128, S)).T

    NLT = D // 128
    FPS = C // NT2
    dep = []
    last = [None]
    PINW = 128
    LAG = 3

    def conv_gen(fr0, never):
        for c in range(NLT):
            ls = slice(c * 128, (c + 1) * 128)
            for half in range(FPS // 8):
                fre = pl.ds(pl.multiple_of(fr0 + half * 8, 8), 8)
                fim = pl.ds(pl.multiple_of(fr0 + half * 8 + C + _PAD, 8), 8)
                fimy = pl.ds(pl.multiple_of(fr0 + half * 8 + C, 8), 8)
                prev = None
                for b in range(NB):
                    ar = ai = None
                    for m in range(b + 1):
                        hr = hh_s[m, fre, ls]
                        if dep:
                            hr = jnp.where(never, dep.pop(), hr)
                        hi = hh_s[m, fim, ls]
                        ur = u_s[b - m, fre, ls]
                        ui = u_s[b - m, fim, ls]
                        pr = hr * ur - hi * ui
                        pi = hr * ui + hi * ur
                        ar = pr if ar is None else ar + pr
                        ai = pi if ai is None else ai + pi
                        last[0] = ar
                        yield
                    if prev is None:
                        yr, yi = ar, ai
                    else:
                        yr = ar - prev[1]
                        yi = ai + prev[0]
                    prev = (ar, ai)
                    y_s[b, fre, ls] = yr
                    y_s[b, fimy, ls] = yi
                    last[0] = yr

    NPAIR = NLT * (FPS // 8) * (NB * (NB + 1) // 2)

    def p2(i, carry):
        r = rows(i, TM2)
        rh = rows(i, TM2 // 2)
        never = jax.lax.broadcasted_iota(jnp.int32, (8, 128), 0) > (i + 8)
        gen = conv_gen(i * FPS, never)
        never16 = jax.lax.broadcasted_iota(jnp.int32, (16, 128), 0) > (i + 16)
        hist = []
        npieces = (FH // 128) * (S // KC)
        per = -(-NPAIR // npieces)

        def pump(d):
            dep.append(d[0:8, 0:128])
            for _ in range(per):
                next(gen, None)
            hist.append(last[0])

        bias = bcol_s[r, :]
        for n in range(FH // 128):
            ns = slice(n * 128, (n + 1) * 128)
            acc = None
            for kc in range(S // KC):
                lhs = wsp_v[r, kc * KC:(kc + 1) * KC]
                if LAG and len(hist) >= LAG:
                    t = jnp.concatenate([hist[-LAG]] * 2, axis=0).astype(bf16)
                    cols = []
                    for c0 in range(0, KC, 128):
                        if c0 < PINW:
                            a0 = jnp.where(never16, t, lhs[0:16, c0:c0 + 128])
                            cols.append(jnp.concatenate([a0, lhs[16:, c0:c0 + 128]], axis=0))
                        else:
                            cols.append(lhs[:, c0:c0 + 128])
                    lhs = cols[0] if len(cols) == 1 else jnp.concatenate(cols, axis=1)
                d = jnp.dot(lhs, _unpack(z2_s[kc * KC // 2:(kc + 1) * KC // 2, ns]),
                            preferred_element_type=f32)
                acc = d if acc is None else acc + d
                pump(d)
            p_s[rh, ns] = _pack((_unpack(z1_s[rh, ns]).astype(f32) * (acc + bias)).astype(bf16))
        for _ in gen:
            pass
        return carry

    with jax.named_scope('p2'):
        jax.lax.fori_loop(0, NT2, p2, 0, unroll=4)

    def out_copy(i):
        r = rows(i, C)
        return pltpu.make_async_copy(o_s.at[r], o_hbm.at[r], sem_o.at[i])

    def p3(i, carry):
        gm = g_v[...]
        dd = d_v[...].astype(f32).reshape(1, D)
        gate = _silu(jnp.dot(_unpack(p_s[rows(i, TM3 // 2), :]), wout_v[...], preferred_element_type=f32))
        for bb in range(TM3 // C):
            b = i * (TM3 // C) + bb
            rr = rows(b, C)
            rrh = rows(b, C // 2)
            y = jnp.dot(gm, y_s[b].astype(bf16), preferred_element_type=f32)
            y = y + _unpack(kv_s[rrh, :]).astype(f32) * dd
            s = _unpack(xn_s[rrh, :]).astype(f32) * y
            o_s[rr, :] = (x_v[rr, :].astype(f32) + s * gate[bb * C:(bb + 1) * C]).astype(bf16)
            out_copy(b).start()
        return carry

    with jax.named_scope('p3'):
        jax.lax.fori_loop(0, NT3, p3, 0, unroll=4)
    with jax.named_scope('p4'):
        for i in range(NB):
            out_copy(i).wait()


@jax.jit
def pallas_recurrent_scan__ssm_conv_h3__mixer_gmlp__prompt_kernel(
    A_q: jax.Array,
    A_k: jax.Array,
    A_v: jax.Array,
    A_shift_k: jax.Array,
    A_ssm_k: jax.Array,
    A_ssm_D: jax.Array,
    B_x: jax.Array,
    B_w_in: jax.Array,
    B_w_sp: jax.Array,
    B_b_sp: jax.Array,
    B_w_out: jax.Array,
):
    del B_x
    _, S, D = A_q.shape
    F = B_w_in.shape[-1]
    FH = F // 2
    C = _C
    NB = S // C
    bf16, f32, u32 = jnp.bfloat16, jnp.float32, jnp.uint32

    x = A_q.reshape(S, D)
    k = A_k.reshape(S, D)
    v = A_v.reshape(S, D)
    shk = A_shift_k.T
    dvec = A_ssm_D
    bvec = B_b_sp
    fmat = np.asarray(_F_NP, dtype=np.float32).astype(bf16)
    gmat = np.asarray(_F_NP.T / C, dtype=np.float32).astype(bf16)

    kern = functools.partial(_kernel, S=S, D=D, FH=FH)
    any_spec = pl.BlockSpec(memory_space=pl.ANY)
    out = pl.pallas_call(
        kern,
        out_shape=jax.ShapeDtypeStruct((S, D), bf16),
        in_specs=[any_spec] * 12,
        out_specs=any_spec,
        scratch_shapes=[
            pltpu.VMEM((S, D), bf16),
            pltpu.VMEM((S + 16, D), bf16),
            pltpu.VMEM((S, D), bf16),
            pltpu.VMEM(shk.shape, bf16),
            pltpu.VMEM((D, S), bf16),
            pltpu.VMEM((D,), bf16),
            pltpu.VMEM((D, F), bf16),
            pltpu.VMEM((S, S), bf16),
            pltpu.VMEM((S,), bf16),
            pltpu.VMEM((FH, D), bf16),
            pltpu.VMEM((2 * C, C), bf16),
            pltpu.VMEM((C, 2 * C), bf16),
            pltpu.VMEM((S // 2, D), u32),
            pltpu.VMEM((S // 2, D), u32),
            pltpu.VMEM((S // 2, FH), u32),
            pltpu.VMEM((S // 2, FH), u32),
            pltpu.VMEM((NB, 2 * C + 2 * _PAD, D), f32),
            pltpu.VMEM((NB, 2 * C + 2 * _PAD, D), f32),
            pltpu.VMEM((NB, 2 * C, D), f32),
            pltpu.VMEM((S, D), bf16),
            pltpu.VMEM((S // 2, FH), u32),
            pltpu.VMEM((S, 128), f32),
            pltpu.VMEM((D // 128, _TM1 + 8, 128), f32),
            pltpu.SemaphoreType.DMA((5, S // _TM1)),
            pltpu.SemaphoreType.DMA((7,)),
            pltpu.SemaphoreType.DMA((NB,)),
            pltpu.SemaphoreType.DMA((2,)),
        ],
        compiler_params=pltpu.CompilerParams(vmem_limit_bytes=120 * 1024 * 1024),
    )(x, k, v, shk, A_ssm_k, dvec, B_w_in, B_w_sp, bvec, B_w_out, fmat, gmat)
    return out.reshape(1, S, D)
```

```python
import functools

import jax
import jax.numpy as jnp
import numpy as np
import jax.experimental.pallas as pl
import jax.experimental.pallas.tpu as pltpu

_C = 128
_TM1 = 256
_TM2 = 128
_TM3 = 512
_PAD = 8
_KC = 256


def _dft_matrix():
    c = _C
    f = np.concatenate([np.arange(0, c, 2), np.arange(1, c, 2)])
    t = np.arange(c)
    m = ((2 * f[:, None] + 1) * t[None, :]) % (4 * c)
    th = np.pi * m.astype(np.float64) / (2 * c)
    sg = np.where(f % 2 == 0, 1.0, -1.0)[:, None]
    return np.concatenate([np.cos(th), -sg * np.sin(th)], axis=0)


_F_NP = _dft_matrix()


def _ln(x, scale=1.0):
    m = jnp.mean(x, axis=-1, keepdims=True)
    xc = x - m
    v = jnp.mean(xc * xc, axis=-1, keepdims=True)
    return xc * (jax.lax.rsqrt(v + 1e-5) * scale)


def _gelu_half(h):
    c0 = 0.7978845608028654
    return h + h * jnp.tanh(h * (2.0 * c0 + (8.0 * c0 * 0.044715) * (h * h)))


def _silu(x):
    return 0.5 * x * (1.0 + jnp.tanh(0.5 * x))


def _pack(x):
    return pltpu.bitcast(x, jnp.uint32)


def _unpack(x):
    return pltpu.bitcast(x, jnp.bfloat16)


def _kernel(x_hbm, k_hbm, v_hbm, shk_hbm, h_hbm, d_hbm, win_hbm, wsp_hbm, b_hbm, wout_hbm, f_hbm, g_hbm,
            o_hbm,
            x_v, k_v, v_v, shk_v, h_v, d_v, win_v, wsp_v, b_v, wout_v, f_v, g_v,
            xn_s, kv_s, z1_s, z2_s, u_s, hh_s, y_s, o_s, p_s, bcol_s, kf_s,
            sem_t, sem_m, sem_o, sem_w,
            *, S, D, FH):
    C, TM1, TM2, TM3, KC = _C, _TM1, _TM2, _TM3, _KC
    NT1, NT2, NT3 = S // TM1, S // TM2, S // TM3
    NB = S // C
    f32, bf16 = jnp.float32, jnp.bfloat16

    def rows(i, n):
        if isinstance(i, int):
            return pl.ds(i * n, n)
        return pl.ds(pl.multiple_of(i * n, n), n)

    def put(ref, b, val):
        ref[b, 0:C, :] = val[:C]
        ref[b, C + _PAD:2 * C + _PAD, :] = val[C:]

    def tile_copies(i):
        r = rows(i, TM1)
        return [
            None,
            pltpu.make_async_copy(k_hbm.at[r], k_v.at[pl.ds(pl.multiple_of(i * TM1 + 16, 16), TM1)], sem_t.at[1, i]),
            pltpu.make_async_copy(v_hbm.at[r], v_v.at[r], sem_t.at[2, i]),
            pltpu.make_async_copy(h_hbm.at[:, r], h_v.at[:, r], sem_t.at[3, i]),
        ]

    def wsp_copy(i):
        r = rows(i, TM1)
        return pltpu.make_async_copy(wsp_hbm.at[r], wsp_v.at[r], sem_t.at[4, i])

    misc = [
        None,
        pltpu.make_async_copy(shk_hbm, shk_v, sem_m.at[1]),
        pltpu.make_async_copy(f_hbm, f_v, sem_m.at[2]),
        pltpu.make_async_copy(d_hbm, d_v, sem_m.at[3]),
        pltpu.make_async_copy(b_hbm, b_v, sem_m.at[4]),
        pltpu.make_async_copy(wout_hbm, wout_v, sem_m.at[5]),
        pltpu.make_async_copy(g_hbm, g_v, sem_m.at[6]),
    ]

    x_copy = lambda i: pltpu.make_async_copy(x_hbm.at[rows(i, TM1)], x_v.at[rows(i, TM1)], sem_t.at[0, i])
    kvh_copies = lambda i: tile_copies(i)[1:]
    def win_copy(c):
        c0 = (1 - c) * FH
        return pltpu.make_async_copy(win_hbm.at[:, pl.ds(c0, FH)], win_v.at[:, pl.ds(c0, FH)], sem_w.at[c])

    def once(fn):
        jax.lax.fori_loop(0, 1, lambda i, c: (fn(), c)[1], 0)

    x_copy(0).start()
    win_copy(0).start()
    k_v[pl.ds(0, 16), :] = jnp.zeros((16, D), bf16)
    with jax.named_scope("p0"):
        x_copy(0).wait()
    win_copy(1).start()
    xn_s[rows(0, TM1 // 2), :] = _pack(_ln(x_v[rows(0, TM1), :].astype(f32), 0.5).astype(bf16))
    win_copy(0).wait()
    misc[1].start()
    misc[2].start()
    for c in kvh_copies(0):
        c.start()
    x_copy(1).start()

    def first_a():
        xn = _unpack(xn_s[rows(0, TM1 // 2), :])
        z2 = _gelu_half(jnp.dot(xn, win_v[:, FH:], preferred_element_type=f32))
        z2_s[rows(0, TM1 // 2), :] = _pack(_ln(z2).astype(bf16))

    with jax.named_scope("p0b"):
        once(first_a)
    win_copy(1).wait()
    for c in misc[3:]:
        c.start()

    misc[1].wait()
    misc[2].wait()

    def p1(i, carry, first=False):
        def nxt():
            for c in kvh_copies(i + 1):
                c.start()
            x_copy(i + 1).wait()

        if first:
            nxt()
            x_copy(2).start()
        else:
            pl.when(i + 1 < NT1)(nxt)
            pl.when(i + 2 < NT1)(lambda: x_copy(i + 2).start())

        wsp_copy(i).start()
        for c in kvh_copies(i):
            c.wait()
        r = rows(i, TM1)
        rh = rows(i, TM1 // 2)
        r0 = i * TM1 if first else pl.multiple_of(i * TM1, TM1)
        never = jax.lax.broadcasted_iota(jnp.int32, (8, 128), 0) > (i + 8)

        def anchor(val, d):
            a0 = jnp.where(never, d[0:8, 0:128].astype(val.dtype), val[0:8, 0:128])
            top = jnp.concatenate([a0, val[8:, 0:128]], axis=0)
            return top if val.shape[1] == 128 else jnp.concatenate([top, val[:, 128:]], axis=1)

        never16 = jax.lax.broadcasted_iota(jnp.int32, (16, 128), 0) > (i + 16)
        pins = {}

        def pinned(lhs, j):
            if j not in pins or first:
                return lhs
            t = None
            for pv in pins[j]:
                for c0 in range(0, pv.shape[1], 128):
                    for rr0 in range(0, pv.shape[0], 8 * PST):
                        q = pv[rr0:rr0 + 8, c0:c0 + 128]
                        t = q if t is None else jnp.maximum(t, q)
            t = jnp.concatenate([t, t], axis=0).astype(bf16)
            cols = []
            for c0 in range(0, lhs.shape[1], 128):
                a0 = jnp.where(never16, t, lhs[0:16, c0:c0 + 128])
                cols.append(jnp.concatenate([a0, lhs[16:, c0:c0 + 128]], axis=0))
            return cols[0] if len(cols) == 1 else jnp.concatenate(cols, axis=1)

        PST = 1
        PL = 4
        NZ = FH // 128
        BPT = TM1 // C
        fm = f_v[...]
        xn = _unpack(xn_s[rh, :])
        shk = shk_v[...].astype(f32)
        j = 0
        z2 = []
        kvs = []
        KVP = [3, 3, 5, 12, 13]

        def do_kv(n, anc):
            ls = slice(n * 128, (n + 1) * 128)
            kk = k_v[pl.ds(r0, TM1 + 16), ls].astype(f32)
            if anc is not None:
                kk = anchor(kk, anc)
            kf_s[n] = kk[8:]
            ks = kk[16:16 + TM1] * shk[0:1, ls]
            for t in range(1, 4):
                ks = ks + kf_s[n, 8 - t:8 - t + TM1, :] * shk[t:t + 1, ls]
            kvn = ks * v_v[r, ls].astype(f32)
            pins.setdefault(KVP[n], []).append(kvn)
            kvn = kvn.astype(bf16)
            kv_s[rh, ls] = _pack(kvn)
            kvs.append(kvn)

        def do_h(bb):
            hb = h_v[:, rows(i * BPT + bb, C)]
            put(hh_s, i * BPT + bb, jax.lax.dot_general(pinned(fm, j), hb, (((1,), (1,)), ((), ())),
                                                        preferred_element_type=f32))

        do_h(0)
        j += 1
        do_kv(0, None)
        do_kv(1, None)
        if first:
            for n in range(2, D // 128):
                do_kv(n, None)
        for n in range(0 if first else NZ):
            d = jnp.dot(pinned(xn, j), win_v[:, FH + n * 128:FH + (n + 1) * 128], preferred_element_type=f32)
            gl = _gelu_half(d)
            z2.append(gl)
            pins.setdefault(j + PL, []).append(gl)
            if n == 1:
                do_kv(2, d)
            j += 1
        do_h(1)
        j += 1
        if first:
            xx = _ln(x_v[rows(1, TM1), :].astype(f32), 0.5)
            xn_s[rows(1, TM1 // 2), :] = _pack(xx.astype(bf16))
        else:
            zl = _ln(jnp.concatenate(z2, axis=1))
            z2_s[rh, :] = _pack(zl.astype(bf16))
            pins.setdefault(j + 3, []).append(zl)
        for n in range(NZ):
            d = jnp.dot(pinned(xn, j), win_v[:, n * 128:(n + 1) * 128], preferred_element_type=f32)
            gl = _gelu_half(d)
            z1_s[rh, n * 128:(n + 1) * 128] = _pack(gl.astype(bf16))
            pins.setdefault(j + PL, []).append(gl)
            if n == 1 and not first:
                do_kv(3, d)
            if n == 2 and not first:
                do_kv(4, d)
            if n == 4 and not first:
                inx = jnp.minimum(i + 1, NT1 - 1)
                xx = _ln(anchor(x_v[rows(inx, TM1), :].astype(f32), d), 0.5)
                xn_s[rows(inx, TM1 // 2), :] = _pack(xx.astype(bf16))
            j += 1
        kv = jnp.concatenate(kvs, axis=1)
        for bb in range(BPT):
            b = i * BPT + bb
            put(u_s, b, jnp.dot(pinned(fm, j), kv[bb * C:(bb + 1) * C, :], preferred_element_type=f32))
            j += 1
        return carry

    with jax.named_scope('p1'):
        with jax.named_scope('p1a'):
            p1(0, 0, first=True)
        jax.lax.fori_loop(1, NT1, p1, 0, unroll=1)
    with jax.named_scope('p1b'):
        for c in misc[3:]:
            c.wait()
        for i in range(NT1):
            wsp_copy(i).wait()

    bcol_s[...] = jnp.broadcast_to(b_v[...].astype(f32).reshape(1, S), (128, S)).T

    NLT = D // 128
    FPS = C // NT2
    dep = []
    last = [None]
    PINW = 128
    LAG = 3

    def conv_gen(fr0, never):
        for c in range(NLT):
            ls = slice(c * 128, (c + 1) * 128)
            for half in range(FPS // 8):
                fre = pl.ds(pl.multiple_of(fr0 + half * 8, 8), 8)
                fim = pl.ds(pl.multiple_of(fr0 + half * 8 + C + _PAD, 8), 8)
                fimy = pl.ds(pl.multiple_of(fr0 + half * 8 + C, 8), 8)
                prev = None
                for b in range(NB):
                    ar = ai = None
                    for m in range(b + 1):
                        hr = hh_s[m, fre, ls]
                        if dep:
                            hr = jnp.where(never, dep.pop(), hr)
                        hi = hh_s[m, fim, ls]
                        ur = u_s[b - m, fre, ls]
                        ui = u_s[b - m, fim, ls]
                        pr = hr * ur - hi * ui
                        pi = hr * ui + hi * ur
                        ar = pr if ar is None else ar + pr
                        ai = pi if ai is None else ai + pi
                        last[0] = ar
                        yield
                    if prev is None:
                        yr, yi = ar, ai
                    else:
                        yr = ar - prev[1]
                        yi = ai + prev[0]
                    prev = (ar, ai)
                    y_s[b, fre, ls] = yr
                    y_s[b, fimy, ls] = yi
                    last[0] = yr

    NPAIR = NLT * (FPS // 8) * (NB * (NB + 1) // 2)

    def p2(i, carry):
        r = rows(i, TM2)
        rh = rows(i, TM2 // 2)
        never = jax.lax.broadcasted_iota(jnp.int32, (8, 128), 0) > (i + 8)
        gen = conv_gen(i * FPS, never)
        never16 = jax.lax.broadcasted_iota(jnp.int32, (16, 128), 0) > (i + 16)
        hist = []
        npieces = (FH // 128) * (S // KC)
        per = -(-NPAIR // npieces)

        def pump(d):
            dep.append(d[0:8, 0:128])
            for _ in range(per):
                next(gen, None)
            hist.append(last[0])

        bias = bcol_s[r, :]
        for n in range(FH // 128):
            ns = slice(n * 128, (n + 1) * 128)
            acc = None
            for kc in range(S // KC):
                lhs = wsp_v[r, kc * KC:(kc + 1) * KC]
                if LAG and len(hist) >= LAG:
                    t = jnp.concatenate([hist[-LAG]] * 2, axis=0).astype(bf16)
                    cols = []
                    for c0 in range(0, KC, 128):
                        if c0 < PINW:
                            a0 = jnp.where(never16, t, lhs[0:16, c0:c0 + 128])
                            cols.append(jnp.concatenate([a0, lhs[16:, c0:c0 + 128]], axis=0))
                        else:
                            cols.append(lhs[:, c0:c0 + 128])
                    lhs = cols[0] if len(cols) == 1 else jnp.concatenate(cols, axis=1)
                d = jnp.dot(lhs, _unpack(z2_s[kc * KC // 2:(kc + 1) * KC // 2, ns]),
                            preferred_element_type=f32)
                acc = d if acc is None else acc + d
                pump(d)
            p_s[rh, ns] = _pack((_unpack(z1_s[rh, ns]).astype(f32) * (acc + bias)).astype(bf16))
        for _ in gen:
            pass
        return carry

    with jax.named_scope('p2'):
        jax.lax.fori_loop(0, NT2, p2, 0, unroll=4)

    def out_copy(i):
        r = rows(i, C)
        return pltpu.make_async_copy(o_s.at[r], o_hbm.at[r], sem_o.at[i])

    def p3(i, carry):
        gm = g_v[...]
        dd = 2.0 * d_v[...].astype(f32).reshape(1, D)
        gate = _silu(jnp.dot(_unpack(p_s[rows(i, TM3 // 2), :]), wout_v[...], preferred_element_type=f32))
        for bb in range(TM3 // C):
            b = i * (TM3 // C) + bb
            rr = rows(b, C)
            rrh = rows(b, C // 2)
            y = jnp.dot(gm, y_s[b].astype(bf16), preferred_element_type=f32)
            y = y + _unpack(kv_s[rrh, :]).astype(f32) * dd
            s = _unpack(xn_s[rrh, :]).astype(f32) * y
            o_s[rr, :] = (x_v[rr, :].astype(f32) + s * gate[bb * C:(bb + 1) * C]).astype(bf16)
            out_copy(b).start()
        return carry

    with jax.named_scope('p3'):
        jax.lax.fori_loop(0, NT3, p3, 0, unroll=4)
    with jax.named_scope('p4'):
        for i in range(NB):
            out_copy(i).wait()


@jax.jit
def pallas_recurrent_scan__ssm_conv_h3__mixer_gmlp__prompt_kernel(
    A_q: jax.Array,
    A_k: jax.Array,
    A_v: jax.Array,
    A_shift_k: jax.Array,
    A_ssm_k: jax.Array,
    A_ssm_D: jax.Array,
    B_x: jax.Array,
    B_w_in: jax.Array,
    B_w_sp: jax.Array,
    B_b_sp: jax.Array,
    B_w_out: jax.Array,
):
    del B_x
    _, S, D = A_q.shape
    F = B_w_in.shape[-1]
    FH = F // 2
    C = _C
    NB = S // C
    bf16, f32, u32 = jnp.bfloat16, jnp.float32, jnp.uint32

    x = A_q.reshape(S, D)
    k = A_k.reshape(S, D)
    v = A_v.reshape(S, D)
    shk = A_shift_k.T
    dvec = A_ssm_D
    bvec = B_b_sp
    fmat = np.asarray(_F_NP, dtype=np.float32).astype(bf16)
    gmat = np.asarray(_F_NP.T * (2.0 / C), dtype=np.float32).astype(bf16)

    kern = functools.partial(_kernel, S=S, D=D, FH=FH)
    any_spec = pl.BlockSpec(memory_space=pl.ANY)
    out = pl.pallas_call(
        kern,
        out_shape=jax.ShapeDtypeStruct((S, D), bf16),
        in_specs=[any_spec] * 12,
        out_specs=any_spec,
        scratch_shapes=[
            pltpu.VMEM((S, D), bf16),
            pltpu.VMEM((S + 16, D), bf16),
            pltpu.VMEM((S, D), bf16),
            pltpu.VMEM(shk.shape, bf16),
            pltpu.VMEM((D, S), bf16),
            pltpu.VMEM((D,), bf16),
            pltpu.VMEM((D, F), bf16),
            pltpu.VMEM((S, S), bf16),
            pltpu.VMEM((S,), bf16),
            pltpu.VMEM((FH, D), bf16),
            pltpu.VMEM((2 * C, C), bf16),
            pltpu.VMEM((C, 2 * C), bf16),
            pltpu.VMEM((S // 2, D), u32),
            pltpu.VMEM((S // 2, D), u32),
            pltpu.VMEM((S // 2, FH), u32),
            pltpu.VMEM((S // 2, FH), u32),
            pltpu.VMEM((NB, 2 * C + 2 * _PAD, D), f32),
            pltpu.VMEM((NB, 2 * C + 2 * _PAD, D), f32),
            pltpu.VMEM((NB, 2 * C, D), f32),
            pltpu.VMEM((S, D), bf16),
            pltpu.VMEM((S // 2, FH), u32),
            pltpu.VMEM((S, 128), f32),
            pltpu.VMEM((D // 128, _TM1 + 8, 128), f32),
            pltpu.SemaphoreType.DMA((5, S // _TM1)),
            pltpu.SemaphoreType.DMA((7,)),
            pltpu.SemaphoreType.DMA((NB,)),
            pltpu.SemaphoreType.DMA((2,)),
        ],
        compiler_params=pltpu.CompilerParams(vmem_limit_bytes=120 * 1024 * 1024),
    )(x, k, v, shk, A_ssm_k, dvec, B_w_in, B_w_sp, bvec, B_w_out, fmat, gmat)
    return out.reshape(1, S, D)
```
